```python
import os as _os
_os.environ.setdefault("JAX_PLATFORMS", "cpu")
import jax
import jax.numpy as jnp

def _softmax(x, axis=-1):
    return jax.nn.softmax(x, axis=axis)
def _gelu(x):
    return jax.nn.gelu(x, approximate=True)
def _silu(x):
    return jax.nn.silu(x)
def _sigmoid(x):
    return jax.nn.sigmoid(x)
def _layernorm(x, axis=-1, eps=1e-5):
    m = jnp.mean(x, axis=axis, keepdims=True)
    v = jnp.var(x, axis=axis, keepdims=True)
    return (x - m) / jnp.sqrt(v + eps)
def _scatter_add(tgt, idx, src, axis=0):
    return tgt.at[idx].add(src)
def _segment_sum(src, seg, n):
    return jax.ops.segment_sum(src, seg, n)
class _Rng:
    def __init__(self, key):
        self._k = key
    def _next(self):
        self._k, sub = jax.random.split(self._k)
        return sub
    def normal(self, shape):
        return jax.random.normal(self._next(), shape, dtype=jnp.bfloat16)
    def randint(self, lo, hi, shape):
        return jax.random.randint(self._next(), shape, lo, hi, dtype=jnp.int32)
    def uniform(self, shape, lo=0.0, hi=1.0):
        return jax.random.uniform(self._next(), shape, jnp.bfloat16, lo, hi)
    def permutation(self, n):
        return jax.random.permutation(self._next(), n)


kernel_name = 'gated_mix__grouped_kv_mqa__glu_gated_reglu__prompt'

def setup_inputs():
    _rng = _Rng(jax.random.key(int.from_bytes(__import__("os").urandom(4), "little")))
    _w = (lambda a: (lambda t: t.astype(jnp.bfloat16) if jnp.issubdtype(t.dtype, jnp.floating) else t)(jnp.asarray(a)))
    def _A_setup():
        B, S, D, H = 1, 2048, 640, 32
        Dh = D // H
        return {
            "x": _w((lambda *s: _rng.normal(s) * 0.05)(B, S, D)),
            "wq": _w((lambda *s: _rng.normal(s) * 0.2)(D, H * Dh)),
            "wk": _w((lambda *s: _rng.normal(s) * 0.2)(D, Dh)),
            "wv": _w((lambda *s: _rng.normal(s) * 0.05)(D, Dh)),
            "wo": _w((lambda *s: _rng.normal(s) * 0.05)(H * Dh, D)),
        }
    _A_in = _A_setup()

    def _B_setup():
        B, S, D, F = 1, 2048, 640, 1536
        return {
            "x": _w((lambda *s: _rng.normal(s) * 0.05)(B, S, D)),
            "W_gate": _w((lambda *s: _rng.normal(s) * 0.4)(D, F) * (2.0 / D) ** 0.5),
            "W_up": _w((lambda *s: _rng.normal(s) * 0.4)(D, F) * (2.0 / D) ** 0.5),
            "W_down": _w((lambda *s: _rng.normal(s) * 0.4)(F, D) * (1.0 / F) ** 0.5),
        }
    _B_in = _B_setup()

    return {
        "A_x": _A_in["x"],
        "A_wq": _A_in["wq"],
        "A_wk": _A_in["wk"],
        "A_wv": _A_in["wv"],
        "A_wo": _A_in["wo"],
        "B_x": _B_in["x"],
        "B_W_gate": _B_in["W_gate"],
        "B_W_up": _B_in["W_up"],
        "B_W_down": _B_in["W_down"],
        "gate_w": _w((lambda *s: _rng.normal(s) * 0.05)(640) * 16.0),
    }

def reference(A_x, A_wq, A_wk, A_wv, A_wo, B_x, B_W_gate, B_W_up, B_W_down, gate_w):
    def _A_ref(x, wq, wk, wv, wo):
        B, S, D = x.shape
        H = 32
        Dh = D // H
        q = (lambda x, *d: x.transpose(*d))((x @ wq).reshape(B, S, H, Dh), 0, 2, 1, 3)
        k = x @ wk
        v = x @ wv
        scores = jnp.einsum("bhqd,bkd->bhqk", q, k) * (Dh ** -0.5)
        p = _softmax(scores, axis=-1)
        o = jnp.einsum("bhqk,bkd->bhqd", p, v)
        return (lambda x, *d: x.transpose(*d))(o, 0, 2, 1, 3).reshape(B, S, H * Dh) @ wo

    def _B_ref(x, W_gate, W_up, W_down):
        gate = jnp.einsum("bsd,df->bsf", x, W_gate)
        up = jnp.einsum("bsd,df->bsf", x, W_up)
        gate = gate * (lambda x, dt: x.astype(dt))(gate > 0, gate.dtype)
        h = gate * up
        return jnp.einsum("bsf,fd->bsd", h, W_down)

    x = A_x
    g = _sigmoid((x * gate_w).sum(-1, keepdims=True))
    a = _A_ref(x, A_wq, A_wk, A_wv, A_wo)
    b = _B_ref(x, B_W_gate, B_W_up, B_W_down)
    return g * a + (1 - g) * b
```

```python
import functools
import math
import numpy as np
import jax
import jax.numpy as jnp
from jax import lax
import jax.experimental.pallas as pl
import jax.experimental.pallas.tpu as pltpu

S, D, H, DH, F = 2048, 640, 32, 20, 1536
LANES = 128
NT = S // LANES
BF16 = jnp.bfloat16
F32 = jnp.float32
NN = (((1,), (0,)), ((), ()))
NT_DIMS = (((1,), (1,)), ((), ()))


def make(TQ=512, KC=128, UNROLL=2, KDIM=32, VROWS=32, VF32=False, RB=512, FC=512, flags=None):
    TPI = TQ // LANES
    NQB = S // TQ
    NITEMS = NQB * H
    NKC = S // KC
    WROWS = D + 48
    QSCALE = float(DH ** -0.5 * math.log2(math.e))

    def kernel(wkT_ref, wvT_ref, gw_ref, x_hbm, wq_hbm, wo_hbm, wg_hbm, wu_hbm, wd_hbm,
               out_hbm,
               x_v, wq_v, wo_v, wg_v, wu_v, wd_v, wT, qT, kpad, vT, gT, s0, s1, oT, o_v, sems, osems):
        XC = 512
        nxc = S // XC
        cp_wq = pltpu.make_async_copy(wq_hbm, wq_v, sems.at[0])
        cp_x = [pltpu.make_async_copy(x_hbm.at[pl.ds(i * XC, XC)], x_v.at[pl.ds(i * XC, XC)], sems.at[1 + i])
                for i in range(nxc)]
        cp_w = [pltpu.make_async_copy(a, b, sems.at[1 + nxc + i])
                for i, (a, b) in enumerate([(wg_hbm, wg_v), (wu_hbm, wu_v), (wd_hbm, wd_v), (wo_hbm, wo_v)])]
        cp_wq.start()
        for c in cp_x:
            c.start()
        for c in cp_w:
            c.start()

        gw = gw_ref[...].astype(F32)
        grow = jnp.concatenate([gw[i:i + 1, :] for i in range(D // LANES)], axis=1)
        tail = jnp.concatenate([wkT_ref[...].astype(F32), jnp.zeros((4, D), F32),
                                wvT_ref[...].astype(F32), grow, jnp.zeros((3, D), F32)], axis=0)
        wT[pl.ds(D, 48), :] = tail.astype(BF16)
        cp_wq.wait()
        wT[pl.ds(0, D), :] = wq_v[...].T

        for i in range(nxc):
            cp_x[i].wait()
            xc = x_v[pl.ds(i * XC, XC), :]
            r = lax.dot_general(wT[...], xc, NT_DIMS, preferred_element_type=F32)
            for t in range(XC // LANES):
                tt = i * (XC // LANES) + t
                rt = r[:, t * LANES:(t + 1) * LANES]
                qT[tt, pl.ds(0, D), :] = rt[:D] * QSCALE
                qT[tt, pl.ds(D, 16), :] = jnp.zeros((16, LANES), F32)
                kt = jnp.concatenate([rt[D:D + 24], jnp.zeros((LANES - 24, LANES), F32)], axis=0)
                kpad[pl.ds(tt * LANES, LANES), :] = kt.T.astype(BF16)
                vt = rt[D + 24:D + 48]
                row = lax.broadcasted_iota(jnp.int32, (24, LANES), 0)
                gl = vt[20:21]
                gT[tt] = jnp.broadcast_to(1.0 / (1.0 + jnp.exp(-gl)), (8, LANES))
                vt = jnp.where(row < DH, vt, jnp.where(row == DH, 1.0, 0.0))
                if VF32:
                    vt = vt.astype(BF16).astype(F32)
                    vT[tt] = vt
                else:
                    if VROWS > 24:
                        vt = jnp.concatenate([vt, jnp.zeros((VROWS - 24, LANES), F32)], axis=0)
                    vT[tt] = vt.astype(BF16)

        def load_q(item):
            qb = item // H
            h = item % H
            row = lax.broadcasted_iota(jnp.int32, (32, LANES), 0)
            tiles = []
            for t in range(TPI):
                q = qT[qb * TPI + t, pl.ds(h * DH, 32), :]
                q = jnp.where(row < DH, q, 0.0).astype(BF16)
                if KDIM > 32:
                    q = jnp.concatenate([q, jnp.zeros((KDIM - 32, LANES), BF16)], axis=0)
                tiles.append(q)
            return jnp.concatenate(tiles, axis=1)

        def stage_a(q, sbuf, c, m):
            k = kpad[pl.ds(c * KC, KC), :]
            if KDIM < LANES:
                k = k[:, :KDIM]
            s = lax.dot_general(k, q, NN, preferred_element_type=F32)
            sbuf[pl.ds(c * KC, KC), :] = s
            mc = jnp.max(s.reshape(KC // 8, 8, TQ), axis=0)
            return mc if m is None else jnp.maximum(m, mc)

        def stage_b(sbuf, c, m, acc):
            for j in range(KC // LANES):
                kt = c * (KC // LANES) + j
                s = sbuf[pl.ds(kt * LANES, LANES), :]
                p = jnp.exp2(s.reshape(LANES // 8, 8, TQ) - m[None]).reshape(LANES, TQ).astype(BF16)
                o = lax.dot_general(vT[kt], p, NN, preferred_element_type=F32)
                o = o[:24]
                acc = o if acc is None else acc + o
            return acc

        def finish_m(m):
            return jnp.broadcast_to(jnp.max(m, axis=0, keepdims=True), (8, TQ))

        def finish_o(item, acc):
            qb = item // H
            h = item % H
            for t in range(TPI):
                a = acc[:, t * LANES:(t + 1) * LANES]
                g = gT[qb * TPI + t]
                sc = g[0:1] / a[DH:DH + 1]
                oT[qb * TPI + t, pl.ds(h * DH, 24), :] = a * sc

        def step(item_a, buf_a, item_b, buf_b, m_b):
            q = load_q(item_a) if item_a is not None else None
            m = None
            acc = None
            for c in range(NKC):
                if item_a is not None:
                    m = stage_a(q, buf_a, c, m)
                if item_b is not None:
                    acc = stage_b(buf_b, c, m_b, acc)
            if item_b is not None:
                finish_o(item_b, acc)
            return finish_m(m) if item_a is not None else None

        m0 = step(0, s0, None, None, None)
        bufs = (s0, s1)

        def body(j, m):
            for u in range(UNROLL):
                i = j * UNROLL + u
                m = step(i + 1, bufs[(u + 1) % 2], i, bufs[u % 2], m)
            return m

        nloop = (NITEMS - 1) // UNROLL
        m = lax.fori_loop(0, nloop, body, m0)
        for i in range(nloop * UNROLL, NITEMS - 1):
            m = step(i + 1, bufs[(i + 1) % 2], i, bufs[i % 2], m)
        step(None, None, NITEMS - 1, bufs[(NITEMS - 1) % 2], m)

        for c in cp_w:
            c.wait()

        def ffn(rb, carry):
            r0 = pl.multiple_of(rb * RB, RB)
            xb = x_v[pl.ds(r0, RB), :]
            os_, gs = [], []
            for t in range(RB // LANES):
                tt = rb * (RB // LANES) + t
                os_.append(oT[tt, pl.ds(0, D), :].T.astype(BF16))
                gs.append(jnp.broadcast_to(gT[tt][0:1], (LANES, LANES)).T)
            o = jnp.concatenate(os_, axis=0)
            omg = 1.0 - jnp.concatenate(gs, axis=0)
            acc = None
            for f in range(F // FC):
                gate = jnp.dot(xb, wg_v[:, pl.ds(f * FC, FC)], preferred_element_type=F32)
                up = jnp.dot(xb, wu_v[:, pl.ds(f * FC, FC)], preferred_element_type=F32)
                hh = (jnp.maximum(gate, 0.0) * up).astype(BF16)
                d = jnp.dot(hh, wd_v[pl.ds(f * FC, FC), :], preferred_element_type=F32)
                acc = d if acc is None else acc + d
            a = jnp.dot(o, wo_v[...], preferred_element_type=F32)
            res = a + jnp.concatenate([omg] * (D // LANES), axis=1) * acc
            o_v[pl.ds(r0, RB), :] = res.astype(BF16)
            pltpu.make_async_copy(o_v.at[pl.ds(r0, RB)], out_hbm.at[pl.ds(r0, RB)], osems.at[rb]).start()
            return carry

        lax.fori_loop(0, S // RB, ffn, 0)
        for rb in range(S // RB):
            pltpu.make_async_copy(o_v.at[pl.ds(rb * RB, RB)], out_hbm.at[pl.ds(rb * RB, RB)], osems.at[rb]).wait()

    vmem = pl.BlockSpec(memory_space=pltpu.VMEM)
    hbm = pl.BlockSpec(memory_space=pl.ANY)
    call = pl.pallas_call(
        kernel,
        out_shape=jax.ShapeDtypeStruct((S, D), BF16),
        in_specs=[vmem, vmem, vmem, hbm, hbm, hbm, hbm, hbm, hbm],
        out_specs=hbm,
        scratch_shapes=[
            pltpu.VMEM((S, D), BF16), pltpu.VMEM((D, D), BF16), pltpu.VMEM((D, D), BF16),
            pltpu.VMEM((D, F), BF16), pltpu.VMEM((D, F), BF16), pltpu.VMEM((F, D), BF16),
            pltpu.VMEM((WROWS, D), BF16),
            pltpu.VMEM((NT, D + 16, LANES), F32),
            pltpu.VMEM((S, LANES), BF16),
            pltpu.VMEM((NT, 24 if VF32 else VROWS, LANES), F32 if VF32 else BF16),
            pltpu.VMEM((NT, 8, LANES), F32),
            pltpu.VMEM((S, TQ), F32), pltpu.VMEM((S, TQ), F32),
            pltpu.VMEM((NT, D + 8, LANES), F32),
            pltpu.VMEM((S, D), BF16),
            pltpu.SemaphoreType.DMA((9,)),
            pltpu.SemaphoreType.DMA((S // RB,)),
        ],
        compiler_params=pltpu.CompilerParams(vmem_limit_bytes=100 * 2**20, flags=flags),
        name="gated_mix",
    )

    def fn(A_x, A_wq, A_wk, A_wv, A_wo, B_x, B_W_gate, B_W_up, B_W_down, gate_w):
        out = call(A_wk.T, A_wv.T, gate_w.reshape(D // LANES, LANES), A_x.reshape(S, D), A_wq, A_wo,
                   B_W_gate, B_W_up, B_W_down)
        return out.reshape(1, S, D)
    return jax.jit(fn)


_impl = make(VF32=True, UNROLL=4)


@jax.jit
def pallas_gated_mix__grouped_kv_mqa__glu_gated_reglu__prompt_kernel(
    A_x, A_wq, A_wk, A_wv, A_wo, B_x, B_W_gate, B_W_up, B_W_down, gate_w,
):
    return _impl(A_x, A_wq, A_wk, A_wv, A_wo, B_x, B_W_gate, B_W_up, B_W_down, gate_w)
```

```python
import math
import jax
import jax.numpy as jnp
from jax import lax
import jax.experimental.pallas as pl
import jax.experimental.pallas.tpu as pltpu

S, D, H, DH, F = 2048, 640, 32, 20, 1536
LANES = 128
NT = S // LANES
ND = D // LANES
NF = F // LANES
BF16 = jnp.bfloat16
F32 = jnp.float32
U32 = jnp.uint32
HG = 4
NI = H // HG


def plan(mrows, n_ffn, delta, fend, minq, minpv, nres, foff, gr=16):
    tot = sum(mrows)
    ends = [i * tot + sum(mrows[:c + 1]) for i in range(NI) for c in range(NT)]
    total_att = NI * (tot + NT * 24)
    prog, t, att_t, row, nf, nxt, last_pv = [], 0, 0, 0, 0, 0, -10**6
    ripe = []
    while row < NI * tot or ripe:
        done = row == NI * tot
        due = max(ripe[0][0], last_pv + minpv) if ripe else None
        if ripe and due <= t:
            k = ripe.pop(0)[1]
            prog.append(("pv", k // NT, k % NT)); last_pv = t; t += 24; att_t += 24
            continue
        behind = nf < n_ffn - nres and (nf - foff) / (n_ffn - nres) <= att_t / (total_att * fend)
        if behind and prog and prog[-1][0] == "pv" and not done:
            n = minq
        elif (behind and prog) or done:
            if nf < n_ffn:
                prog.append(("ffn", nf)); nf += 1; t += 128
            else:
                t = due
            continue
        elif ripe:
            n = max(minq, -(-(due - t) // gr) * gr)
        else:
            n = -(-(ends[nxt] - row + delta) // gr) * gr
        n = min(n, NI * tot - row)
        prog.append(("qk", row, row + n))
        while nxt < len(ends) and ends[nxt] <= row + n:
            ripe.append((t + ends[nxt] - row + delta, nxt)); nxt += 1
        t += n; att_t += n; row += n
    prog += [("ffn", k) for k in range(nf, n_ffn)]
    return prog


def make(PAT=((3,),), L0=3, DELTA=168, FEND=1.0, FOFF=0.0, NRES=4, MINQ=16, MINPV=96, PF32=True,
         XQ=False, XACC=False, XGU=False, XH=False, XB=False, VLAST=False, REV=False, FB=True, XCH=(2, 14),
         LIMIT=3600.0, SC=False, PADR=32, OTR=32, VTR=0, flags=None, name="gated_mix"):
    vg = [PAT[t % len(PAT)] for t in range(NT)]
    goff = [sum(sum(v) for v in vg[:t]) for t in range(NT + 1)]
    mrows = [LANES - 8 * sum(g) for g in vg]
    moff = [sum(mrows[:t]) for t in range(NT + 1)]
    tot = moff[NT]
    WROWS = D + 48
    QSCALE = float(DH ** -0.5 * math.log2(math.e))
    xst = [sum(XCH[:i]) for i in range(len(XCH) + 1)]

    def kernel(wkT_hbm, wvT_hbm, gw_hbm, x_hbm, wq_hbm, wo_hbm, wg_hbm, wu_hbm, wd_hbm,
               out_hbm,
               wkv_v, gw_v,
               x_v, wq_v, wo_v, wg_v, wu_v, wd_v, wT, xT, qT, qp32, kpad, kp32, ka32, vT, gT, kb, oT, o_v, h32, s_v,
               sems, osems, *bufs):
        accb, gub, bb = (bufs[:4], bufs[4:8]), bufs[8:12], (bufs[12:17], bufs[17:22])
        nxc = len(XCH)
        copies = [(wkT_hbm, wkv_v.at[0]), (wvT_hbm, wkv_v.at[1]), (gw_hbm, gw_v.at[0])]
        xcp = [(x_hbm.at[pl.ds(xst[i] * LANES, XCH[i] * LANES)],
                x_v.bitcast(BF16).at[pl.ds(xst[i] * LANES, XCH[i] * LANES)]) for i in range(nxc)]
        copies += xcp[:1] + [(wq_hbm.at[pl.ds(n * LANES, LANES)], wq_v.bitcast(BF16).at[pl.ds(n * LANES, LANES)])
                             for n in range(ND)] + xcp[1:]
        copies += [(a, b.bitcast(BF16)) for a, b in [(wg_hbm, wg_v), (wu_hbm, wu_v), (wd_hbm, wd_v), (wo_hbm, wo_v)]]
        copies = [pltpu.make_async_copy(a, b, sems.at[i]) for i, (a, b) in enumerate(copies)]
        for c in copies:
            c.start()
        b16 = lambda v: pltpu.bitcast(v, BF16)
        mm = lambda a, b: jnp.dot(a, b, preferred_element_type=F32)
        u32 = lambda v: pltpu.bitcast(v.astype(BF16), U32)

        def wait(cs, nm):
            if SC:
                with jax.named_scope(nm):
                    for c in cs:
                        c.wait()
            else:
                for c in cs:
                    c.wait()

        wait(copies[:3], 'w_small')
        gw = gw_v[0].astype(F32)
        grow = jnp.concatenate([gw[i:i + 1, :] for i in range(ND)], axis=1)
        tail = jnp.concatenate([wkv_v[0].astype(F32), jnp.zeros((4, D), F32),
                                wkv_v[1].astype(F32), grow, jnp.zeros((3, D), F32)], axis=0)
        for n in range(ND):
            wT[n, pl.ds(0, 48), :] = tail[:, n * LANES:(n + 1) * LANES].astype(BF16)

        def transpose_x(i):
            for tt in range(xst[i], xst[i + 1]):
                xT[tt] = b16(x_v[pl.ds(tt * LANES // 2, LANES // 2), :]).T

        wait(copies[3:4], 'w_x0')
        transpose_x(0)
        for n in range(ND):
            wait(copies[4 + n:5 + n], 'w_wq%d' % n)
            wT[n, pl.ds(48, D), :] = b16(wq_v[pl.ds(n * 64, 64), :]).T

        qmax = kmax = vmax = jnp.zeros((8, LANES), F32)
        for i in range(nxc):
            if i:
                wait(copies[8 + i:9 + i], 'w_x%d' % i)
                transpose_x(i)
            for tt in range(xst[i], xst[i + 1]):
                rt = jnp.concatenate([
                    mm(jnp.concatenate([b16(wT.bitcast(U32)[n, pl.ds(a // 2, (b - a) // 2), :]) for n in range(ND)], axis=1),
                       b16(xT.bitcast(U32)[tt])) for a, b in ((0, 176), (176, 352), (352, 528), (528, WROWS))], axis=0)
                qT[tt, pl.ds(0, D), :] = rt[48:] * QSCALE
                qT[tt, pl.ds(D, 16), :] = jnp.zeros((16, LANES), F32)
                row = lax.broadcasted_iota(jnp.int32, (32, LANES), 0)
                for h in range(H):
                    q = jnp.where(row < DH, qT[tt, pl.ds(h * DH, 32), :], 0.0)
                    qp32[tt, pl.ds(h * 16, 16), :] = u32(q)
                    qmax = jnp.maximum(qmax, jnp.sum(q[:24] * q[:24], axis=0, keepdims=True))
                kt = rt[:24]
                kmax = jnp.maximum(kmax, jnp.sum(kt * kt, axis=0, keepdims=True))
                kk = jnp.concatenate([kt, jnp.zeros((LANES - 24, LANES), F32)], axis=0).T
                ka32[pl.ds(tt * 64, 64), :] = u32(kk)
                nv = sum(vg[tt]) * 8
                kv, km = (kk[LANES - nv:], kk[:LANES - nv]) if VLAST and nv else (kk[:max(nv, 8)], kk[nv:])
                kpad[pl.ds(moff[tt], mrows[tt]), :] = km
                if nv:
                    for d in range(DH):
                        kd = jnp.broadcast_to(kv[:, d:d + 1], (nv, LANES))
                        o_ = 0
                        for va in vg[tt]:
                            kb[pl.ds(((goff[tt] + o_) * DH + d * va) * 8, va * 8), :] = kd[o_ * 8:(o_ + va) * 8]
                            o_ += va
                vt = rt[24:48]
                row = lax.broadcasted_iota(jnp.int32, (24, LANES), 0)
                gT[tt] = jnp.broadcast_to(1.0 / (1.0 + jnp.exp(-vt[DH:DH + 1])), (8, LANES))
                vt = jnp.where(row < DH, vt, 0.0)
                vmax = jnp.maximum(vmax, jnp.max(jnp.abs(vt).reshape(3, 8, LANES), axis=0))
                vT[pl.ds(tt * 24, 24), :] = jnp.where(row == DH, 1.0, vt).astype(BF16).astype(F32)

        kp32[pl.ds(0, tot // 2), :] = u32(kpad[pl.ds(0, tot), :])
        vtop = jnp.max(vmax)
        bounded = (jnp.max(qmax) * jnp.max(kmax) <= LIMIT) & (vtop <= 2.0 ** 40) & (vtop >= 2.0 ** -40)
        wait(copies[8 + nxc:], 'w_ffn')

        def store_head(j, h, o):
            oT[pl.ds(h * DH, 24), :] = o * (gT[j][0:1] / o[DH:DH + 1])

        def out_copy(j):
            r0 = pl.multiple_of(j * LANES, LANES)
            return pltpu.make_async_copy(o_v.at[pl.ds(r0, LANES)], out_hbm.at[pl.ds(r0, LANES)], osems.at[j])

        def shifted_tile(j, carry):
            def item(i, carry):
                q = [b16(qp32[j, pl.ds(pl.multiple_of((i * HG + u) * 16, 16), 16), :]) for u in range(HG)]
                s = mm(b16(ka32[...])[:, :32], jnp.concatenate(q, axis=1))
                s_v[...] = s
                top = jnp.max(s, axis=0, keepdims=True)
                v = jnp.concatenate([vT[pl.ds(c * 24, 24), :] for c in range(NT)], axis=1)
                o = mm(v, jnp.exp2(s_v[...] - top))
                for u in range(HG):
                    store_head(j, i * HG + u, o[:, u * LANES:(u + 1) * LANES])
                return carry

            lax.fori_loop(0, NI, item, 0)
            xb = b16(x_v[pl.ds(pl.multiple_of(j * (LANES // 2), LANES // 2), LANES // 2), :])
            hid = jnp.maximum(mm(xb, b16(wg_v[...])), 0.0) * mm(xb, b16(wu_v[...]))
            omg = 1.0 - jnp.broadcast_to(gT[j][0:1], (LANES, LANES)).T
            res = (mm(oT[pl.ds(0, D), :].T.astype(BF16), b16(wo_v[...]))
                   + jnp.concatenate([omg] * ND, axis=1) * mm(hid.astype(BF16), b16(wd_v[...])))
            o_v[pl.ds(pl.multiple_of(j * LANES, LANES), LANES), :] = res.astype(BF16)
            out_copy(j).start()
            return carry

        def bounded_tile(j, carry):
            r0 = pl.multiple_of(j * LANES, LANES)
            r0h = pl.multiple_of(j * (LANES // 2), LANES // 2)
            st = {}
            always = qT[j, pl.ds(D, 8), :] == 0.0
            zs = {}

            def zero(key):
                if key not in zs:
                    zs[key] = pl.multiple_of(((j + len(zs)) >> 12) << 5, 32)
                return zs[key]

            def t_qk(a, b):
                for i in range(NI):
                    lo, hi = max(a, i * tot) - i * tot, min(b, (i + 1) * tot) - i * tot
                    if lo >= hi:
                        continue
                    z = zero(("qk", a) if XQ else ("i", i))
                    k = b16(kp32[pl.ds(z + lo // 2, (hi - lo) // 2), :])[:, :32]
                    for h in range(i * HG, (i + 1) * HG):
                        q = b16(qp32[j, pl.ds(z + h * 16, 16), :])
                        e = jnp.exp2(mm(k, q))
                        for c in range(NT):
                            l2, h2 = max(lo, moff[c]), min(hi, moff[c + 1])
                            if l2 < h2:
                                st.setdefault(("p", h, c), []).append(e[l2 - lo:h2 - lo])

            def vpu_group(h, g0, va):
                acc = None
                for d in range(DH):
                    kk = kb[pl.ds(zero(("h", h)) + (g0 * DH + d * va) * 8, va * 8), :]
                    qq = qT[j, pl.ds(zero(("g", h // HG, g0)) + h * DH + d, 8, stride=0), :]
                    if d == L0 and "lnk" in st:
                        qq = jnp.where(always, qq, st["lnk"])
                    pr = kk.reshape(va, 8, LANES) * qq[None]
                    acc = pr if acc is None else acc + pr
                src = [acc[n] for n in range(va)]
                while len(src) > 1:
                    src = src[2:] + [jnp.maximum(src[0], src[1])]
                st["lnk"] = src[0]
                return jnp.exp2(acc).reshape(va * 8, LANES)

            def t_pv(i, c):
                v = vT[pl.ds(zero(("i", i)) + c * 24, 24), :]
                vp = {}
                for u in (range(HG - 1, -1, -1) if REV else range(HG)):
                    vp[u] = [vpu_group(i * HG + u, goff[c] + sum(vg[c][:g]), va) for g, va in enumerate(vg[c])]
                for u in range(HG):
                    h = i * HG + u
                    mp = st.pop(("p", h, c))
                    p = jnp.concatenate(mp + vp[u] if VLAST else vp[u] + mp, axis=0)
                    if not PF32:
                        p = p.astype(BF16)
                    o = lax.dot_general(v, p, (((1,), (0,)), ((), ())), preferred_element_type=F32)
                    if c:
                        o = o + (accb[(c + 1) % 2][u][pl.ds(zero(("i", i)), 24), :] if XACC else st["acc", h])
                    if c == NT - 1:
                        store_head(j, h, o)
                    elif XACC:
                        accb[c % 2][u][pl.ds(0, 24), :] = o
                    else:
                        st["acc", h] = o

            def t_gu(f, s_):
                z = zero(("gu", f, s_))
                if s_ < 4:
                    w = (wg_v, wu_v)[s_ // 2]
                    xb = b16(x_v[pl.ds(z + r0h, LANES // 2), pl.ds(0, 512)])
                    r = mm(xb, b16(w[pl.ds(0, 256), pl.ds((2 * f + s_ % 2) * LANES, LANES)]))
                    if XGU:
                        gub[s_][...] = r
                    else:
                        st["gu", s_] = r
                else:
                    xb = b16(x_v[pl.ds(z + r0h, LANES // 2), pl.ds(512, LANES)])
                    part = [gub[n][pl.ds(z, LANES), :] if XGU else st.pop(("gu", n)) for n in range(4)]
                    g = mm(xb, b16(wg_v[pl.ds(256, 64), pl.ds(f * 256, 256)])) + jnp.concatenate(part[:2], axis=1)
                    u = mm(xb, b16(wu_v[pl.ds(256, 64), pl.ds(f * 256, 256)])) + jnp.concatenate(part[2:], axis=1)
                    hid = jnp.maximum(g, 0.0) * u
                    if XH:
                        for n in range(2):
                            h32[2 * f + n] = u32(hid[:, n * LANES:(n + 1) * LANES])
                    else:
                        st["h", f] = hid

            def one_minus_g():
                if "omg" not in st:
                    st["omg"] = 1.0 - jnp.broadcast_to(gT[j][0:1], (LANES, LANES)).T
                return st["omg"]

            def t_down(kq, n):
                z = zero(("d", kq, n))
                if XH:
                    hb = jnp.concatenate([b16(h32[4 * kq + m, pl.ds(z, LANES // 2), :]) for m in range(4)], axis=1)
                else:
                    if ("hb", kq) not in st:
                        st["hb", kq] = jnp.concatenate([st.pop(("h", 2 * kq)), st.pop(("h", 2 * kq + 1))], axis=1).astype(BF16)
                    hb = st["hb", kq]
                d = mm(hb, b16(wd_v[pl.ds(kq * 256, 256), pl.ds(n * LANES, LANES)]))
                if XB:
                    if kq:
                        d = d + bb[(kq + 1) % 2][n][pl.ds(z, LANES), :]
                    if kq == 2:
                        d = d * one_minus_g()
                    bb[kq % 2][n][...] = d
                else:
                    st["d", kq, n] = d
                    if n == ND - 1:
                        d = jnp.concatenate([st.pop(("d", kq, m)) for m in range(ND)], axis=1)
                        st["b"] = d if kq == 0 else st["b"] + d

            def t_wo(n):
                if "o" not in st:
                    st["o"] = oT[pl.ds(0, 512), :].T.astype(BF16)
                r = mm(st["o"], b16(wo_v[pl.ds(0, 256), pl.ds(n * LANES, LANES)]))
                if XB:
                    bb[1][n][...] = r + bb[0][n][pl.ds(zero(("wo", n)), LANES), :]
                else:
                    st["a", n] = r

            def t_out():
                ot = oT[pl.ds(512, LANES), :].T
                l4 = mm(ot.astype(BF16), b16(wo_v[pl.ds(256, 64), pl.ds(0, 512)]))
                l1 = jnp.concatenate([mm(ot[32 * r:32 * r + 32].astype(BF16), b16(wo_v[pl.ds(256, 64), pl.ds(512, LANES)]))
                                      for r in range(4)], axis=0)
                if XB:
                    b = jnp.concatenate([bb[1][n][pl.ds(zero("out"), LANES), :] for n in range(ND)], axis=1)
                else:
                    b = (jnp.concatenate([one_minus_g()] * ND, axis=1) * st["b"]
                         + jnp.concatenate([st.pop(("a", n)) for n in range(ND)], axis=1))
                o_v[pl.ds(r0, LANES), :] = (b + jnp.concatenate([l4, l1], axis=1)).astype(BF16)

            ffn = []
            for kq in range(3):
                ffn += [(t_gu, (2 * kq + f, s_)) for f in range(2) for s_ in range(5)]
                if kq:
                    ffn += [(t_down, (kq - 1, n)) for n in range(ND)]
            ffn += [(t_down, (2, n)) for n in range(ND)]
            ffn += [(t_wo, (n,)) for n in range(ND)]
            for it in plan(mrows, len(ffn), DELTA, FEND, MINQ, MINPV, NRES, FOFF):
                if it[0] == "qk":
                    t_qk(*it[1:])
                elif it[0] == "pv":
                    t_pv(*it[1:])
                else:
                    ffn[it[1]][0](*ffn[it[1]][1])
            t_out()
            out_copy(j).start()
            return carry

        if FB:
            @pl.when(bounded)
            def _():
                lax.fori_loop(0, NT, bounded_tile, 0)

            @pl.when(jnp.logical_not(bounded))
            def _():
                lax.fori_loop(0, NT, shifted_tile, 0)
        else:
            lax.fori_loop(0, NT, bounded_tile, 0)

        wait([out_copy(j) for j in range(NT)], 'w_out')

    hbm = pl.BlockSpec(memory_space=pl.ANY)
    call = pl.pallas_call(
        kernel,
        out_shape=jax.ShapeDtypeStruct((S, D), BF16),
        in_specs=[hbm] * 9,
        out_specs=hbm,
        scratch_shapes=[
            pltpu.VMEM((8, DH, D), BF16), pltpu.VMEM((PADR // 4, ND, LANES), BF16),
            pltpu.VMEM((S // 2, D), U32), pltpu.VMEM((D // 2, D), U32), pltpu.VMEM((D // 2, D), U32),
            pltpu.VMEM((D // 2, F), U32), pltpu.VMEM((D // 2, F), U32), pltpu.VMEM((F // 2, D), U32),
            pltpu.VMEM((ND, 704, LANES), BF16),
            pltpu.VMEM((NT, D, LANES), BF16),
            pltpu.VMEM((NT, D + 32, LANES), F32),
            pltpu.VMEM((NT, H * 16, LANES), U32),
            pltpu.VMEM((S, LANES), F32),
            pltpu.VMEM((S // 2, LANES), U32),
            pltpu.VMEM((S // 2, LANES), U32),
            pltpu.VMEM((NT * 24, LANES), F32),
            pltpu.VMEM((NT, 8, LANES), F32),
            pltpu.VMEM((-(-DH * max(goff[NT], 1) * 8 // 32) * 32, LANES), F32),
            pltpu.VMEM((D + OTR, LANES), F32),
            pltpu.VMEM((S, D), BF16),
            pltpu.VMEM((NF, LANES // 2, LANES), U32),
            pltpu.VMEM((S, HG * LANES), F32),
            pltpu.SemaphoreType.DMA((12 + len(XCH),)),
            pltpu.SemaphoreType.DMA((NT,)),
        ] + [pltpu.VMEM((32, LANES), F32)] * 8 + [pltpu.VMEM((LANES, LANES), F32)] * 14,
        compiler_params=pltpu.CompilerParams(vmem_limit_bytes=100 * 2**20, internal_scratch_in_bytes=96 * 512, flags=flags),
        name=name,
    )

    def fn(A_x, A_wq, A_wk, A_wv, A_wo, B_x, B_W_gate, B_W_up, B_W_down, gate_w):
        out = call(A_wk.T, A_wv.T, gate_w.reshape(ND, LANES), A_x.reshape(S, D), A_wq, A_wo,
                   B_W_gate, B_W_up, B_W_down)
        return out.reshape(1, S, D)
    return jax.jit(fn)


_impl = make(**dict(XCH=(1,3,12)))


@jax.jit
def pallas_gated_mix__grouped_kv_mqa__glu_gated_reglu__prompt_kernel(
    A_x, A_wq, A_wk, A_wv, A_wo, B_x, B_W_gate, B_W_up, B_W_down, gate_w,
):
    return _impl(A_x, A_wq, A_wk, A_wv, A_wo, B_x, B_W_gate, B_W_up, B_W_down, gate_w)
```

```python
import functools
import math

import jax
import jax.numpy as jnp
from jax import lax
import jax.experimental.pallas as pl
import jax.experimental.pallas.tpu as pltpu

S, D, H, DH, F = 2048, 640, 32, 20, 1536
L = 128
NT = S // L
ND = D // L
HG = 4
NI = H // HG
HD = DH // 2
VR = 24
BF16, F32, U32 = jnp.bfloat16, jnp.float32, jnp.uint32

MAX_SCORE = 72.0
MAX_VALUE = 2.0 ** 30


def _q_row(head, feature):
    return (feature // HD * 2 + head % 2) * (D // 4) + head // 2 * HD + feature % HD


def _plan(mxu_rows, slots, wait, min_rows, min_gap, reserve, lag):
    per_item = sum(mxu_rows)
    total = NI * per_item
    ends = [i * per_item + sum(mxu_rows[:c + 1]) for i in range(NI) for c in range(NT)]
    att_total = total + NI * NT * VR
    ffn_total = sum(cycles for cycles, _ in slots[:len(slots) - reserve])
    prog, ripe, pv_at = [], [], []
    t = att = ffn = row = slot = tile = 0
    while row < total or ripe:
        due = max(ripe[0], pv_at[-1] + min_gap if pv_at else 0) if ripe else None
        if ripe and due <= t:
            ripe.pop(0)
            prog.append(("pv", len(pv_at) // NT, len(pv_at) % NT))
            pv_at.append(t)
            t, att = t + VR, att + VR
            continue
        need = slots[slot][1] if slot < len(slots) else None
        free = need == 0 or (need and len(pv_at) >= need and pv_at[need - 1] + 400 <= t)
        behind = (free and bool(prog) and slot < len(slots) - reserve
                  and (ffn + lag) / ffn_total <= att / att_total)
        if behind and prog[-1][0] == "pv" and row < total:
            n = min_rows
        elif behind or row == total:
            if free:
                prog.append(("ffn", slot))
                t, ffn, slot = t + slots[slot][0], ffn + slots[slot][0], slot + 1
            else:
                t = due
            continue
        elif ripe:
            n = max(min_rows, -(-(due - t) // 16) * 16)
        else:
            n = -(-(ends[tile] - row + wait) // 16) * 16
        n = min(n, total - row)
        prog.append(("qk", row, row + n))
        while tile < len(ends) and ends[tile] <= row + n:
            ripe.append(t + ends[tile] - row + wait)
            tile += 1
        t, att, row = t + n, att + n, row + n
    return prog + [("ffn", n) for n in range(slot, len(slots))]


def _mm(a, b):
    return jnp.dot(a, b, preferred_element_type=F32)


def _unpack(v):
    return pltpu.bitcast(v, BF16)


def _pack(v):
    return pltpu.bitcast(v.astype(BF16), U32)


def _top(acc):
    return functools.reduce(jnp.maximum, [acc[r:r + 8] for r in range(0, acc.shape[0], 8)])


def make(NB=9, HT=24, WAIT=176, MIN_ROWS=48, MIN_GAP=96, RESERVE=6, LAG=51.2, SKEW=(0, 0, 16, 16),
         LINK=3, AHEAD_LINK=2, XCH=(2, 5, 9), FORD=1, LIMIT=MAX_SCORE ** 2, QUICK=False):
    units = [(b, half, a) for b in range(NB) for half in range(2) for a in range(3)]
    cut = [0] + [max(0, (t * (len(units) + 2) + NT // 2) // NT - 2) for t in range(1, NT + 1)]
    vpu_rows = [units[cut[t]:cut[t + 1]] for t in range(NT)]
    mxu_rows = [L - 8 * len(vpu_rows[t]) - (16 if t == 0 else 0) for t in range(NT)]
    start = [sum(mxu_rows[:t]) for t in range(NT + 1)]
    per_item = start[NT]
    x_at = [sum(XCH[:i]) for i in range(len(XCH) + 1)]
    QG = D // 8 + 2

    def kernel(wk_hbm, wv_hbm, gw_hbm, x_hbm, wq_hbm, wo_hbm, wg_hbm, wu_hbm, wd_hbm, out_hbm,
               wkv_v, gw_v, x_v, wq_v, wo_v, wg_v, wu_v, wd_v, wg0_v, wT, xT, q_v, k_all, k_mxu,
               k_vpu, k_ahead, vT, gT, p_first, p_ahead, gate0, oT, out_v, q_one, s_v, sems, *bufs):
        o_acc, gu_acc, out_acc = (bufs[:4], bufs[4:8]), bufs[8:12], (bufs[12:17], bufs[17:22])

        def fetch(sem, *pairs):
            copies = [pltpu.make_async_copy(src, dst, sems.at[sem]) for src, dst in pairs]
            for c in copies:
                c.start()
            return lambda: [c.wait() for c in copies]

        def x_chunk(i):
            rows = pl.ds(x_at[i] * L, XCH[i] * L)
            return x_hbm.at[rows], x_v.bitcast(BF16).at[rows]

        small_ready = fetch(0, (wk_hbm, wkv_v.at[0]), (wv_hbm, wkv_v.at[1]), (gw_hbm, gw_v.at[0]))
        x_ready = [fetch(1, x_chunk(0))]
        wq_ready = [fetch(2 + n, (wq_hbm.at[pl.ds(n * L, L)], wq_v.bitcast(BF16).at[pl.ds(n * L, L)]))
                    for n in range(ND)]
        x_ready += [fetch(7, x_chunk(1)),
                    fetch(8, x_chunk(2), (wg_hbm.at[pl.ds(0, 4 * L), pl.ds(0, L)], wg0_v.bitcast(BF16)))]
        weights_ready = fetch(9, *((src, dst.bitcast(BF16)) for src, dst in (
            (wg_hbm, wg_v), (wu_hbm, wu_v), (wd_hbm, wd_v), (wo_hbm, wo_v))))

        small_ready()
        gw = gw_v[0].astype(F32)
        head = jnp.concatenate([
            wkv_v[0].astype(F32), jnp.zeros((4, D), F32), wkv_v[1].astype(F32),
            jnp.concatenate([gw[n:n + 1] for n in range(ND)], axis=1), jnp.zeros((3, D), F32)], axis=0)
        for n in range(ND):
            wT[n, pl.ds(0, 48), :] = head[:, n * L:(n + 1) * L].astype(BF16)
        nil = pl.multiple_of(jnp.max(jnp.where(gw > jnp.inf, 1.0, 0.0)).astype(jnp.int32) << 5, 32)

        def transpose_x(t):
            xT[t] = _pack(_unpack(x_v[pl.ds(t * L // 2, L // 2), :]).T)

        x_ready[0]()
        for t in range(XCH[0]):
            transpose_x(t)
        order = sorted(range(2 * H), key=lambda a: _q_row(a // 2, a % 2 * HD))
        for n in range(ND):
            wq_ready[n]()
            w = _pack(_unpack(wq_v[pl.ds(n * L // 2, L // 2), :]).T)
            wT[n, pl.ds(48, D), :] = _unpack(jnp.concatenate([w[5 * a:5 * a + 5] for a in order], axis=0))

        def q_tile(j, offset=0):
            return q_v.at[pl.ds(j * QG + offset, QG)]

        def q_feature(q, row, side=0):
            return q[row // 8, pl.ds(row % 8, 1), pl.ds(side * L, L)]

        def chained(always, q_row, link):
            return q_row if link is None else jnp.where(always, q_row, link)

        def times(k, q):
            return k * (q if q.shape[0] == 1 else jnp.concatenate([q] * (k.shape[0] // 8), axis=0))

        def first_keys(q, k, h, always, link, link_at):
            acc = None
            for d in range(DH):
                qd = q_feature(q, _q_row(h, d))
                term = times(k[d], chained(always, qd, link) if d == link_at else qd)
                acc = term if acc is None else acc + term
            return jnp.exp2(acc), _top(acc)

        link = None

        def first_keys_of(t, heads):
            always = q_tile(0)[D // 8, :, pl.ds(0, L)] == 0.0
            out = link
            for h in heads:
                p, out = first_keys(q_tile(t), k_ahead, h, always, out, 0)
                if h < HT:
                    p_first[h] = p
                else:
                    p_ahead[t, h - HT] = p
            return out

        q_norm = k_norm = v_peak = jnp.zeros((8, L), F32)
        wT32 = wT.bitcast(U32)
        phase = [0, x_at[1], x_at[2] - 1, NT]
        for i in range(3):
            if i:
                x_ready[i]()
                if phase[i] == x_at[i]:
                    transpose_x(x_at[i])
            for t in range(phase[i], phase[i + 1]):
                xt = _unpack(xT[t, pl.ds(nil, D // 2), :])
                if i and t + 1 < x_at[i + 1]:
                    transpose_x(t + 1)
                proj = jnp.concatenate([
                    _mm(jnp.concatenate([_unpack(wT32[n, pl.ds(a // 2, (b - a) // 2), :]) for n in range(ND)],
                                        axis=1), xt)
                    for a, b in ((0, 176), (176, 352), (352, 528), (528, 48 + D))], axis=0)

                q = proj[48:] * (DH ** -0.5 * math.log2(math.e))
                b11, b12, b21, b22 = (q[m * D // 4:(m + 1) * D // 4] for m in range(4))
                t1 = b12 - b11
                t2 = b22 - t1
                mixed = jnp.concatenate([b21 - t2, t1, t2, b22 - b12], axis=0)
                both = jnp.concatenate([q, mixed], axis=1)
                both = jnp.concatenate([both, jnp.zeros((16, 2 * L), F32)], axis=0)
                q_v[pl.ds(t * QG, QG)] = both.reshape(QG, 8, 2 * L)
                sq = q[:D // 2] * q[:D // 2] + q[D // 2:] * q[D // 2:]
                for h in range(H):
                    r = _q_row(h, 0) // 8 * 8
                    q_norm = jnp.maximum(q_norm, sq[r:r + 8] + sq[r + 8:r + 16])

                k = proj[:24]
                k_norm = jnp.maximum(k_norm, jnp.sum(k * k, axis=0, keepdims=True))
                k = jnp.concatenate([k[:HD], jnp.zeros((16 - HD, L), F32), k[HD:DH],
                                     jnp.zeros((L - 16 - HD, L), F32)], axis=0).T
                k_all[pl.ds(t * L, L), :] = k
                if t == 0:
                    for d in range(DH):
                        e = d // HD * 16 + d % HD
                        k_ahead[d] = jnp.broadcast_to(k[:16, e:e + 1], (16, L))
                    k = k[16:]
                if start[t + 1] % 16 == 0:
                    u = max(u for u in range(t + 1) if start[u] % 16 == 0)
                    rows = [k_all[pl.ds((w + 1) * L - mxu_rows[w], mxu_rows[w]), :] for w in range(u, t)]
                    k_mxu[pl.ds(start[u] // 2, (start[t + 1] - start[u]) // 2), :] = _pack(
                        jnp.concatenate(rows + [k[8 * len(vpu_rows[t]):]], axis=0))
                for n, (b, half, a) in enumerate(vpu_rows[t]):
                    for d in range(HD):
                        lo, hi = (jnp.broadcast_to(k[8 * n:8 * n + 8, e:e + 1], (8, L)) for e in (d, d + 16))
                        at = [((b * 7 + m) * HD + d, pl.ds(8 * a, 8)) for m in range(7)]
                        if half == 0:
                            k_vpu[at[0]], k_vpu[at[1]] = lo, hi
                        else:
                            a11, a12 = k_vpu[at[0]], k_vpu[at[1]]
                            s1 = lo + hi
                            s2 = s1 - a11
                            for m, term in enumerate((a12 - s2, hi, s1, s2, a11 - lo), 2):
                                k_vpu[at[m]] = term

                v = proj[24:48]
                row = lax.broadcasted_iota(jnp.int32, (VR, L), 0)
                gT[t] = jnp.broadcast_to(1.0 / (1.0 + jnp.exp(-v[DH:DH + 1])), (8, L))
                v = jnp.where(row < DH, v, 0.0)
                v_peak = jnp.maximum(v_peak, _top(jnp.abs(v)))
                vT[t] = jnp.where(row == DH, 1.0, v).astype(BF16).astype(F32)
                if t == NT - 1:
                    gate0[...] = _mm(_unpack(x_v[:, pl.ds(0, 4 * L)]), _unpack(wg0_v[...]))
                if t and not QUICK:
                    link = first_keys_of(t - 1, range(HT, H))
        if not QUICK:
            link = first_keys_of(NT - 1, range(HT, H))
            first_keys_of(0, range(HT))
        v_top = jnp.max(v_peak)
        bounded = ((8.0 * jnp.max(q_norm) * jnp.max(k_norm) <= LIMIT)
                   & (v_top <= MAX_VALUE) & (v_top >= 1.0 / MAX_VALUE))
        weights_ready()

        def head_q(load):
            row = lax.broadcasted_iota(jnp.int32, (16, L), 0)
            return jnp.concatenate([jnp.where(row < HD, load(d), 0.0) for d in (0, HD)], axis=0)

        def store_head(j, h, o):
            oT[pl.ds(h * DH, VR), :] = o * (gT[j][0:1] / o[DH:DH + 1])

        def tile_rows(j, n=L):
            return pl.ds(pl.multiple_of(j * n, n), n)

        def shifted_tile(j, carry):
            q_one[pl.ds(0, QG * 8), :] = q_tile(j)[:, :, pl.ds(0, L)].reshape(QG * 8, L)

            def item(i, carry):
                q = jnp.concatenate([head_q(lambda d: q_one[pl.ds(i * (HG // 2 * HD) + _q_row(u, d), 16), :])
                                     for u in range(HG)], axis=1)
                s = _mm(k_all[...][:, :32].astype(BF16), q.astype(BF16))
                s_v[...] = s
                row_max = jnp.max(s, axis=0, keepdims=True)
                o = _mm(jnp.concatenate([vT[c] for c in range(NT)], axis=1), jnp.exp2(s_v[...] - row_max))
                for u in range(HG):
                    store_head(j, i * HG + u, o[:, u * L:(u + 1) * L])
                return carry

            lax.fori_loop(0, NI, item, 0)
            x = _unpack(x_v[tile_rows(j, L // 2), :])
            hidden = jnp.maximum(_mm(x, _unpack(wg_v[...])), 0.0) * _mm(x, _unpack(wu_v[...]))
            rest = 1.0 - jnp.broadcast_to(gT[j][0:1], (L, L)).T
            out = (_mm(oT[pl.ds(0, D), :].T.astype(BF16), _unpack(wo_v[...]))
                   + jnp.concatenate([rest] * ND, axis=1) * _mm(hidden.astype(BF16), _unpack(wd_v[...])))
            out_v[tile_rows(j), :] = out.astype(BF16)
            return carry

        def bounded_tile(j, p_carry):
            live, zeros = {}, {}
            always = q_tile(j)[D // 8, :, pl.ds(0, L)] == 0.0

            def zero(key, unit):
                if key not in zeros:
                    zeros[key] = (j + len(zeros)) >> 13
                return pl.multiple_of(zeros[key] * unit, unit)

            def q_window(row, n):
                q = q_tile(j)[pl.ds(row // 8, 3), :, pl.ds(0, L)].reshape(24, L)
                return q[row % 8:row % 8 + n]

            def mxu_scores(row0, row1):
                pieces = []
                for u in range(HG):
                    lo, hi = (r and min(r + SKEW[u], NI * per_item - 16 * sum(e > r for e in qk_ends))
                              for r in (row0, row1))
                    spans = [(i, max(lo, i * per_item), min(hi, (i + 1) * per_item)) for i in range(NI)]
                    pieces.append([(i, a - i * per_item, b - i * per_item) for i, a, b in spans if a < b])
                count = max(len(p) for p in pieces)
                for p in pieces:
                    if len(p) < count:
                        i, a, b = p.pop()
                        p += [(i, a, a + 16), (i, a + 16, b)]
                for m in range(count):
                    for u in range(HG):
                        i, a, b = pieces[u][m]
                        k = _unpack(k_mxu[pl.ds(zero(i, 32) + a // 2, (b - a) // 2), :])[:, :32]
                        if ("q", i, u) not in live:
                            live["q", i, u] = head_q(lambda d: q_window(_q_row(i * HG + u, d), 16)).astype(BF16)
                        p = jnp.exp2(_mm(k, live["q", i, u]))
                        for c in range(NT):
                            lo, hi = max(a, start[c]), min(b, start[c + 1])
                            if lo < hi:
                                live.setdefault(("p", i, u, c), []).append(p[lo - a:hi - a])

            def vpu_scores(i, pair, b):
                k = k_vpu.at[pl.ds(zero(("k", i, pair), 4) + b * 7 * HD, 7 * HD)]
                q = q_tile(j, zero(("q", i, b), 2))

                def product(m, acc, link):
                    quarter, side = ((0, 2, 3)[m], 0) if m < 3 else (m - 3, 1)
                    for d in range(HD):
                        qd = q_feature(q, quarter * (D // 4) + (2 * i + pair) * HD + d, side)
                        term = times(k[m * HD + d], chained(always, qd, link) if d == LINK else qd)
                        acc = term if acc is None else acc + term
                    return acc

                p1 = product(0, None, live.get("link"))
                c11 = product(1, p1, None)
                u2 = product(5, p1, _top(c11))
                u3 = product(6, u2, None)
                c21 = product(3, u3, None)
                p5 = product(4, None, _top(c21))
                c12 = product(2, u2 + p5, None)
                live["link"] = _top(c12)
                for half, u, s in ((0, 0, c11), (0, 1, c12), (1, 0, c21), (1, 1, u3 + p5)):
                    for a in range(3):
                        live["p", i, 2 * pair + u, b, half, a] = jnp.exp2(s[8 * a:8 * a + 8])

            def weigh_values(i, c):
                v = vT[zero(i, 4) + c]
                for b, half, a in vpu_rows[c]:
                    if (half, a) == (0, 0):
                        for pair in range(2):
                            vpu_scores(i, pair, b)
                for u in range(HG):
                    h = i * HG + u
                    p = [live.pop(("p", i, u) + unit) for unit in vpu_rows[c]] + live.pop(("p", i, u, c))
                    if c == 0:
                        p = [p_carry[h] if h < HT else p_ahead[j, h - HT]] + p
                    o = _mm(v, jnp.concatenate(p, axis=0))
                    if c:
                        o = o + o_acc[(c + 1) % 2][u][pl.ds(zero(i, 32), VR), :]
                    if c < NT - 1:
                        o_acc[c % 2][u][pl.ds(0, VR), :] = o
                    else:
                        store_head(j, h, o)

            def weight(ref, k0, nk, n0, nn):
                return _unpack(ref[pl.ds(k0 * L // 2, nk * L // 2), pl.ds(n0 * L, nn * L)])

            def x_tile(key, k0, nk):
                rows = pl.ds(pl.multiple_of(zero(key, 32) + j * (L // 2), 32), L // 2)
                return _unpack(x_v[rows, pl.ds(k0 * L, nk * L)])

            def gate_up(f, n):
                key = ("gu", f, n)
                if n < 4:
                    gu_acc[n][...] = _mm(x_tile(key, 0, 4), weight((wg_v, wu_v)[n // 2], 0, 4, 2 * f + n % 2, 1))
                    return
                x = x_tile(key, 4, 1)
                part = [gate0[tile_rows(j), :] if (f, m) == (0, 0) else gu_acc[m][pl.ds(zero(key, 32), L), :]
                        for m in range(4)]
                gate = _mm(x, weight(wg_v, 4, 1, 2 * f, 2)) + jnp.concatenate(part[:2], axis=1)
                up = _mm(x, weight(wu_v, 4, 1, 2 * f, 2)) + jnp.concatenate(part[2:], axis=1)
                live["h", f] = jnp.maximum(gate, 0.0) * up

            def down(k, n):
                if n == 0:
                    live["hidden"] = jnp.concatenate([live.pop(("h", 2 * k + m)) for m in range(2)],
                                                     axis=1).astype(BF16)
                out = _mm(live["hidden"], weight(wd_v, 4 * k, 4, n, 1))
                if k:
                    out = out + out_acc[(k + 1) % 2][n][pl.ds(zero(("down", k, n), 32), L), :]
                if k == 2:
                    if n == 0:
                        live["rest"] = 1.0 - jnp.broadcast_to(gT[j][0:1], (L, L)).T
                    out = out * live["rest"]
                out_acc[k % 2][n][...] = out

            def project(n):
                if n == 0:
                    live["o"] = oT[pl.ds(0, 4 * L), :].T.astype(BF16)
                out_acc[1][n][...] = (_mm(live["o"], weight(wo_v, 0, 4, n, 1))
                                      + out_acc[0][n][pl.ds(zero(("wo", n), 32), L), :])

            def finish():
                o = oT[pl.ds(4 * L, L), :].T
                last = jnp.concatenate([
                    _mm(o.astype(BF16), weight(wo_v, 4, 1, 0, 4)),
                    jnp.concatenate([_mm(o[r:r + 32].astype(BF16), weight(wo_v, 4, 1, 4, 1))
                                     for r in range(0, L, 32)], axis=0)], axis=1)
                out = jnp.concatenate([out_acc[1][n][pl.ds(zero("out", 32), L), :] for n in range(ND)], axis=1)
                out_v[tile_rows(j), :] = (out + last).astype(BF16)

            ffn = []
            if FORD == 1:
                for k in range(3):
                    ffn += [(gate_up, 2 * k + f, n) for f in range(2) for n in range(5)]
                    ffn += [(down, k, n) for n in range(ND)]
            else:
                ffn += [(gate_up, f, n) for f in range(6) for n in range(5)]
                ffn += [(down, k, n) for k in range(3) for n in range(ND)]
            ffn = ffn[1:]
            slots = [(L, 0)] * len(ffn) + [(L, (NI - 1) * NT)] * ND + [(L + 32, NI * NT)]
            ffn += [(project, n) for n in range(ND)] + [(finish,)]
            prog = _plan(mxu_rows, slots, WAIT, MIN_ROWS, MIN_GAP, RESERVE, LAG)
            qk_ends = [task[2] for task in prog if task[0] == "qk"]
            p_next = []
            for kind, *args in prog:
                if kind == "qk":
                    mxu_scores(*args)
                elif kind == "ffn":
                    run, *where = ffn[args[0]]
                    run(*where)
                else:
                    weigh_values(*args)
                    if args == [NI - 1, NT - 1]:
                        q = q_tile(jnp.minimum(j + 1, NT - 1))
                        for h in range(HT):
                            k = k_ahead.at[pl.ds(zero(("ahead", h), 2), DH)]
                            p, live["link"] = first_keys(q, k, h, always, live["link"], AHEAD_LINK)
                            p_next.append(p)
            pltpu.make_async_copy(out_v.at[tile_rows(j)], out_hbm.at[tile_rows(j)], sems.at[10]).start()
            return p_next

        whole_output = pltpu.make_async_copy(out_v, out_hbm, sems.at[10])

        @pl.when(bounded)
        def _():
            lax.fori_loop(0, NT, bounded_tile, [p_first[h] for h in range(HT)])

        @pl.when(jnp.logical_not(bounded))
        def _():
            lax.fori_loop(0, NT, shifted_tile, 0)
            whole_output.start()

        whole_output.wait()

    vmem = pltpu.VMEM
    call = pl.pallas_call(
        kernel,
        out_shape=jax.ShapeDtypeStruct((S, D), BF16),
        in_specs=[pl.BlockSpec(memory_space=pl.ANY)] * 9,
        out_specs=pl.BlockSpec(memory_space=pl.ANY),
        scratch_shapes=[
            vmem((8, DH, D), BF16),
            vmem((8, ND, L), BF16),
            vmem((S // 2, D), U32),
            vmem((D // 2, D), U32),
            vmem((D // 2, D), U32),
            vmem((D // 2, F), U32),
            vmem((D // 2, F), U32),
            vmem((F // 2, D), U32),
            vmem((2 * L, L), U32),
            vmem((ND, 704, L), BF16),
            vmem((NT, D // 2, L), U32),
            vmem((NT * QG, 8, 2 * L), F32),
            vmem((S, L), F32),
            vmem((S // 2, L), U32),
            vmem((-(-NB * 7 * HD // 4) * 4, 24, L), F32),
            vmem((DH, 16, L), F32),
            vmem((NT, VR, L), F32),
            vmem((NT, 8, L), F32),
            vmem((HT, 16, L), F32),
            vmem((NT, H - HT, 16, L), F32),
            vmem((S, L), F32),
            vmem((D + 32, L), F32),
            vmem((S, D), BF16),
            vmem((D + 32, L), F32),
            vmem((S, HG * L), F32),
            pltpu.SemaphoreType.DMA((11,)),
        ] + [vmem((32, L), F32)] * 8 + [vmem((L, L), F32)] * 14,
        compiler_params=pltpu.CompilerParams(vmem_limit_bytes=100 * 2 ** 20),
        name="gated_mix",
    )

    def fn(A_x, A_wq, A_wk, A_wv, A_wo, B_x, B_W_gate, B_W_up, B_W_down, gate_w):
        out = call(A_wk.T, A_wv.T, gate_w.reshape(ND, L), A_x.reshape(S, D), A_wq, A_wo,
                   B_W_gate, B_W_up, B_W_down)
        return out.reshape(1, S, D)
    return jax.jit(fn)


_impl = make(**dict())


@jax.jit
def pallas_gated_mix__grouped_kv_mqa__glu_gated_reglu__prompt_kernel(
    A_x, A_wq, A_wk, A_wv, A_wo, B_x, B_W_gate, B_W_up, B_W_down, gate_w,
):
    return _impl(A_x, A_wq, A_wk, A_wv, A_wo, B_x, B_W_gate, B_W_up, B_W_down, gate_w)
```

```python
import functools
import math

import jax
import jax.numpy as jnp
from jax import lax
import jax.experimental.pallas as pl
import jax.experimental.pallas.tpu as pltpu

S, D, H, DH, F = 2048, 640, 32, 20, 1536
L = 128
NT = S // L
ND = D // L
HG = 4
NI = H // HG
HD = DH // 2
VR = 24
BF16, F32, U32 = jnp.bfloat16, jnp.float32, jnp.uint32

MAX_SCORE = 72.0
MAX_VALUE = 2.0 ** 30

NB = 9
HT = 24
SKEW = (0, 0, 16, 16)
XCH = (2, 5, 9)

VPU_UNITS = [(b, half, a) for b in range(NB) for half in range(2) for a in range(3)]
CUT = [0] + [max(0, (t * (len(VPU_UNITS) + 2) + NT // 2) // NT - 2) for t in range(1, NT + 1)]
VPU_ROWS = [VPU_UNITS[CUT[t]:CUT[t + 1]] for t in range(NT)]
MXU_ROWS = [L - 8 * len(VPU_ROWS[t]) - (16 if t == 0 else 0) for t in range(NT)]
START = [sum(MXU_ROWS[:t]) for t in range(NT + 1)]
PER_ITEM = START[NT]
X_AT = [sum(XCH[:i]) for i in range(len(XCH) + 1)]
QG = D // 8 + 2


def _q_row(head, feature):
    return (feature // HD * 2 + head % 2) * (D // 4) + head // 2 * HD + feature % HD


def _plan(slots, wait=176, min_rows=48, min_gap=96, reserve=6, lag=51.2):
    total = NI * PER_ITEM
    ends = [i * PER_ITEM + START[c + 1] for i in range(NI) for c in range(NT)]
    att_total = total + NI * NT * VR
    ffn_total = sum(cycles for cycles, _ in slots[:len(slots) - reserve])
    prog, ripe, pv_at = [], [], []
    t = att = ffn = row = slot = tile = 0
    while row < total or ripe:
        due = max(ripe[0], pv_at[-1] + min_gap if pv_at else 0) if ripe else None
        if ripe and due <= t:
            ripe.pop(0)
            prog.append(("pv", len(pv_at) // NT, len(pv_at) % NT))
            pv_at.append(t)
            t, att = t + VR, att + VR
            continue
        need = slots[slot][1] if slot < len(slots) else None
        free = need == 0 or (need and len(pv_at) >= need and pv_at[need - 1] + 400 <= t)
        behind = (free and bool(prog) and slot < len(slots) - reserve
                  and (ffn + lag) / ffn_total <= att / att_total)
        if behind and prog[-1][0] == "pv" and row < total:
            n = min_rows
        elif behind or row == total:
            if free:
                prog.append(("ffn", slot))
                t, ffn, slot = t + slots[slot][0], ffn + slots[slot][0], slot + 1
            else:
                t = due
            continue
        elif ripe:
            n = max(min_rows, -(-(due - t) // 16) * 16)
        else:
            n = -(-(ends[tile] - row + wait) // 16) * 16
        n = min(n, total - row)
        prog.append(("qk", row, row + n))
        while tile < len(ends) and ends[tile] <= row + n:
            ripe.append(t + ends[tile] - row + wait)
            tile += 1
        t, att, row = t + n, att + n, row + n
    return prog + [("ffn", n) for n in range(slot, len(slots))]


def _mm(a, b):
    return jnp.dot(a, b, preferred_element_type=F32)


def _unpack(v):
    return pltpu.bitcast(v, BF16)


def _pack(v):
    return pltpu.bitcast(v.astype(BF16), U32)


def _top(acc):
    return functools.reduce(jnp.maximum, [acc[r:r + 8] for r in range(0, acc.shape[0], 8)])


def _kernel(wk_hbm, wv_hbm, gw_hbm, x_hbm, wq_hbm, wo_hbm, wg_hbm, wu_hbm, wd_hbm, out_hbm,
            wkv_v, gw_v, x_v, wq_v, wo_v, wg_v, wu_v, wd_v, wg0_v, wT, xT, q_v, k_all, k_mxu,
            k_vpu, k_ahead, vT, gT, p_first, p_ahead, gate0, oT, out_v, q_one, s_v, sems, *bufs):
    o_acc, gu_acc, out_acc = (bufs[:4], bufs[4:8]), bufs[8:12], (bufs[12:17], bufs[17:22])

    def fetch(sem, *pairs):
        copies = [pltpu.make_async_copy(src, dst, sems.at[sem]) for src, dst in pairs]
        for c in copies:
            c.start()
        return lambda: [c.wait() for c in copies]

    def x_chunk(i):
        rows = pl.ds(X_AT[i] * L, XCH[i] * L)
        return x_hbm.at[rows], x_v.bitcast(BF16).at[rows]

    small_ready = fetch(0, (wk_hbm, wkv_v.at[0]), (wv_hbm, wkv_v.at[1]), (gw_hbm, gw_v.at[0]))
    x_ready = [fetch(1, x_chunk(0))]
    wq_ready = [fetch(2 + n, (wq_hbm.at[pl.ds(n * L, L)], wq_v.bitcast(BF16).at[pl.ds(n * L, L)]))
                for n in range(ND)]
    x_ready += [fetch(7, x_chunk(1)),
                fetch(8, x_chunk(2), (wg_hbm.at[pl.ds(0, 4 * L), pl.ds(0, L)], wg0_v.bitcast(BF16)))]
    weights_ready = fetch(9, *((src, dst.bitcast(BF16)) for src, dst in (
        (wg_hbm, wg_v), (wu_hbm, wu_v), (wd_hbm, wd_v), (wo_hbm, wo_v))))

    small_ready()
    gw = gw_v[0].astype(F32)
    head = jnp.concatenate([
        wkv_v[0].astype(F32), jnp.zeros((4, D), F32), wkv_v[1].astype(F32),
        jnp.concatenate([gw[n:n + 1] for n in range(ND)], axis=1), jnp.zeros((3, D), F32)], axis=0)
    for n in range(ND):
        wT[n, pl.ds(0, 48), :] = head[:, n * L:(n + 1) * L].astype(BF16)
    nil = pl.multiple_of(jnp.max(jnp.where(gw > jnp.inf, 1.0, 0.0)).astype(jnp.int32) << 5, 32)

    def transpose_x(t):
        xT[t] = _pack(_unpack(x_v[pl.ds(t * L // 2, L // 2), :]).T)

    x_ready[0]()
    for t in range(XCH[0]):
        transpose_x(t)
    order = sorted(range(2 * H), key=lambda a: _q_row(a // 2, a % 2 * HD))
    for n in range(ND):
        wq_ready[n]()
        w = _pack(_unpack(wq_v[pl.ds(n * L // 2, L // 2), :]).T)
        wT[n, pl.ds(48, D), :] = _unpack(jnp.concatenate([w[5 * a:5 * a + 5] for a in order], axis=0))

    def q_tile(j, offset=0):
        return q_v.at[pl.ds(j * QG + offset, QG)]

    def q_feature(q, row, side=0):
        return q[row // 8, pl.ds(row % 8, 1), pl.ds(side * L, L)]

    def chained(always, q_row, link):
        return q_row if link is None else jnp.where(always, q_row, link)

    def times(k, q):
        return k * (q if q.shape[0] == 1 else jnp.concatenate([q] * (k.shape[0] // 8), axis=0))

    def first_keys(q, k, h, always, link, link_at):
        acc = None
        for d in range(DH):
            qd = q_feature(q, _q_row(h, d))
            term = times(k[d], chained(always, qd, link) if d == link_at else qd)
            acc = term if acc is None else acc + term
        return jnp.exp2(acc), _top(acc)

    link = None

    def first_keys_of(t, heads):
        always = q_tile(0)[D // 8, :, pl.ds(0, L)] == 0.0
        out = link
        for h in heads:
            p, out = first_keys(q_tile(t), k_ahead, h, always, out, 0)
            if h < HT:
                p_first[h] = p
            else:
                p_ahead[t, h - HT] = p
        return out

    q_norm = k_norm = v_peak = jnp.zeros((8, L), F32)
    wT32 = wT.bitcast(U32)
    phase = [0, X_AT[1], X_AT[2] - 1, NT]
    for i in range(3):
        if i:
            x_ready[i]()
            if phase[i] == X_AT[i]:
                transpose_x(X_AT[i])
        for t in range(phase[i], phase[i + 1]):
            xt = _unpack(xT[t, pl.ds(nil, D // 2), :])
            if i and t + 1 < X_AT[i + 1]:
                transpose_x(t + 1)
            proj = jnp.concatenate([
                _mm(jnp.concatenate([_unpack(wT32[n, pl.ds(a // 2, (b - a) // 2), :]) for n in range(ND)],
                                    axis=1), xt)
                for a, b in ((0, 176), (176, 352), (352, 528), (528, 48 + D))], axis=0)

            q = proj[48:] * (DH ** -0.5 * math.log2(math.e))
            b11, b12, b21, b22 = (q[m * D // 4:(m + 1) * D // 4] for m in range(4))
            t1 = b12 - b11
            t2 = b22 - t1
            mixed = jnp.concatenate([b21 - t2, t1, t2, b22 - b12], axis=0)
            both = jnp.concatenate([q, mixed], axis=1)
            both = jnp.concatenate([both, jnp.zeros((16, 2 * L), F32)], axis=0)
            q_v[pl.ds(t * QG, QG)] = both.reshape(QG, 8, 2 * L)
            sq = q[:D // 2] * q[:D // 2] + q[D // 2:] * q[D // 2:]
            for h in range(H):
                r = _q_row(h, 0) // 8 * 8
                q_norm = jnp.maximum(q_norm, sq[r:r + 8] + sq[r + 8:r + 16])

            k = proj[:24]
            k_norm = jnp.maximum(k_norm, jnp.sum(k * k, axis=0, keepdims=True))
            k = jnp.concatenate([k[:HD], jnp.zeros((16 - HD, L), F32), k[HD:DH],
                                 jnp.zeros((L - 16 - HD, L), F32)], axis=0).T
            k_all[pl.ds(t * L, L), :] = k
            if t == 0:
                for d in range(DH):
                    e = d // HD * 16 + d % HD
                    k_ahead[d] = jnp.broadcast_to(k[:16, e:e + 1], (16, L))
                k = k[16:]
            if START[t + 1] % 16 == 0:
                u = max(u for u in range(t + 1) if START[u] % 16 == 0)
                rows = [k_all[pl.ds((w + 1) * L - MXU_ROWS[w], MXU_ROWS[w]), :] for w in range(u, t)]
                k_mxu[pl.ds(START[u] // 2, (START[t + 1] - START[u]) // 2), :] = _pack(
                    jnp.concatenate(rows + [k[8 * len(VPU_ROWS[t]):]], axis=0))
            for n, (b, half, a) in enumerate(VPU_ROWS[t]):
                for d in range(HD):
                    lo, hi = (jnp.broadcast_to(k[8 * n:8 * n + 8, e:e + 1], (8, L)) for e in (d, d + 16))
                    at = [((b * 7 + m) * HD + d, pl.ds(8 * a, 8)) for m in range(7)]
                    if half == 0:
                        k_vpu[at[0]], k_vpu[at[1]] = lo, hi
                    else:
                        a11, a12 = k_vpu[at[0]], k_vpu[at[1]]
                        s1 = lo + hi
                        s2 = s1 - a11
                        for m, term in enumerate((a12 - s2, hi, s1, s2, a11 - lo), 2):
                            k_vpu[at[m]] = term

            v = proj[24:48]
            row = lax.broadcasted_iota(jnp.int32, (VR, L), 0)
            gT[t] = jnp.broadcast_to(1.0 / (1.0 + jnp.exp(-v[DH:DH + 1])), (8, L))
            v = jnp.where(row < DH, v, 0.0)
            v_peak = jnp.maximum(v_peak, _top(jnp.abs(v)))
            vT[t] = jnp.where(row == DH, 1.0, v).astype(BF16).astype(F32)
            if t == NT - 1:
                gate0[...] = _mm(_unpack(x_v[:, pl.ds(0, 4 * L)]), _unpack(wg0_v[...]))
            if t:
                link = first_keys_of(t - 1, range(HT, H))
    link = first_keys_of(NT - 1, range(HT, H))
    first_keys_of(0, range(HT))
    v_top = jnp.max(v_peak)
    bounded = ((8.0 * jnp.max(q_norm) * jnp.max(k_norm) <= MAX_SCORE ** 2)
               & (v_top <= MAX_VALUE) & (v_top >= 1.0 / MAX_VALUE))
    weights_ready()

    def head_q(load):
        row = lax.broadcasted_iota(jnp.int32, (16, L), 0)
        return jnp.concatenate([jnp.where(row < HD, load(d), 0.0) for d in (0, HD)], axis=0)

    def store_head(j, h, o):
        oT[pl.ds(h * DH, VR), :] = o * (gT[j][0:1] / o[DH:DH + 1])

    def tile_rows(j, n=L):
        return pl.ds(pl.multiple_of(j * n, n), n)

    def shifted_tile(j, carry):
        q_one[pl.ds(0, QG * 8), :] = q_tile(j)[:, :, pl.ds(0, L)].reshape(QG * 8, L)

        def item(i, carry):
            q = jnp.concatenate([head_q(lambda d: q_one[pl.ds(i * (HG // 2 * HD) + _q_row(u, d), 16), :])
                                 for u in range(HG)], axis=1)
            s = _mm(k_all[...][:, :32].astype(BF16), q.astype(BF16))
            s_v[...] = s
            row_max = jnp.max(s, axis=0, keepdims=True)
            o = _mm(jnp.concatenate([vT[c] for c in range(NT)], axis=1), jnp.exp2(s_v[...] - row_max))
            for u in range(HG):
                store_head(j, i * HG + u, o[:, u * L:(u + 1) * L])
            return carry

        lax.fori_loop(0, NI, item, 0)
        x = _unpack(x_v[tile_rows(j, L // 2), :])
        hidden = jnp.maximum(_mm(x, _unpack(wg_v[...])), 0.0) * _mm(x, _unpack(wu_v[...]))
        rest = 1.0 - jnp.broadcast_to(gT[j][0:1], (L, L)).T
        out = (_mm(oT[pl.ds(0, D), :].T.astype(BF16), _unpack(wo_v[...]))
               + jnp.concatenate([rest] * ND, axis=1) * _mm(hidden.astype(BF16), _unpack(wd_v[...])))
        out_v[tile_rows(j), :] = out.astype(BF16)
        return carry

    def bounded_tile(j, p_carry):
        live, zeros = {}, {}
        always = q_tile(j)[D // 8, :, pl.ds(0, L)] == 0.0

        def zero(key, unit):
            if key not in zeros:
                zeros[key] = (j + len(zeros)) >> 13
            return pl.multiple_of(zeros[key] * unit, unit)

        def q_window(row, n):
            q = q_tile(j)[pl.ds(row // 8, 3), :, pl.ds(0, L)].reshape(24, L)
            return q[row % 8:row % 8 + n]

        def mxu_scores(row0, row1):
            pieces = []
            for u in range(HG):
                lo, hi = (r and min(r + SKEW[u], NI * PER_ITEM - 16 * sum(e > r for e in qk_ends))
                          for r in (row0, row1))
                spans = [(i, max(lo, i * PER_ITEM), min(hi, (i + 1) * PER_ITEM)) for i in range(NI)]
                pieces.append([(i, a - i * PER_ITEM, b - i * PER_ITEM) for i, a, b in spans if a < b])
            count = max(len(p) for p in pieces)
            for p in pieces:
                if len(p) < count:
                    i, a, b = p.pop()
                    p += [(i, a, a + 16), (i, a + 16, b)]
            for m in range(count):
                for u in range(HG):
                    i, a, b = pieces[u][m]
                    k = _unpack(k_mxu[pl.ds(zero(i, 32) + a // 2, (b - a) // 2), :])[:, :32]
                    if ("q", i, u) not in live:
                        live["q", i, u] = head_q(lambda d: q_window(_q_row(i * HG + u, d), 16)).astype(BF16)
                    p = jnp.exp2(_mm(k, live["q", i, u]))
                    for c in range(NT):
                        lo, hi = max(a, START[c]), min(b, START[c + 1])
                        if lo < hi:
                            live.setdefault(("p", i, u, c), []).append(p[lo - a:hi - a])

        def vpu_scores(i, pair, b):
            k = k_vpu.at[pl.ds(zero(("k", i, pair), 4) + b * 7 * HD, 7 * HD)]
            q = q_tile(j, zero(("q", i, b), 2))

            def product(m, acc, link):
                quarter, side = ((0, 2, 3)[m], 0) if m < 3 else (m - 3, 1)
                for d in range(HD):
                    qd = q_feature(q, quarter * (D // 4) + (2 * i + pair) * HD + d, side)
                    term = times(k[m * HD + d], chained(always, qd, link) if d == 3 else qd)
                    acc = term if acc is None else acc + term
                return acc

            p1 = product(0, None, live.get("link"))
            c11 = product(1, p1, None)
            u2 = product(5, p1, _top(c11))
            u3 = product(6, u2, None)
            c21 = product(3, u3, None)
            p5 = product(4, None, _top(c21))
            c12 = product(2, u2 + p5, None)
            live["link"] = _top(c12)
            for half, u, s in ((0, 0, c11), (0, 1, c12), (1, 0, c21), (1, 1, u3 + p5)):
                for a in range(3):
                    live["p", i, 2 * pair + u, b, half, a] = jnp.exp2(s[8 * a:8 * a + 8])

        def weigh_values(i, c):
            v = vT[zero(i, 4) + c]
            for b, half, a in VPU_ROWS[c]:
                if (half, a) == (0, 0):
                    for pair in range(2):
                        vpu_scores(i, pair, b)
            for u in range(HG):
                h = i * HG + u
                p = [live.pop(("p", i, u) + unit) for unit in VPU_ROWS[c]] + live.pop(("p", i, u, c))
                if c == 0:
                    p = [p_carry[h] if h < HT else p_ahead[j, h - HT]] + p
                o = _mm(v, jnp.concatenate(p, axis=0))
                if c:
                    o = o + o_acc[(c + 1) % 2][u][pl.ds(zero(i, 32), VR), :]
                if c < NT - 1:
                    o_acc[c % 2][u][pl.ds(0, VR), :] = o
                else:
                    store_head(j, h, o)

        def weight(ref, k0, nk, n0, nn):
            return _unpack(ref[pl.ds(k0 * L // 2, nk * L // 2), pl.ds(n0 * L, nn * L)])

        def x_tile(key, k0, nk):
            rows = pl.ds(pl.multiple_of(zero(key, 32) + j * (L // 2), 32), L // 2)
            return _unpack(x_v[rows, pl.ds(k0 * L, nk * L)])

        def gate_up(f, n):
            key = ("gu", f, n)
            if n < 4:
                gu_acc[n][...] = _mm(x_tile(key, 0, 4), weight((wg_v, wu_v)[n // 2], 0, 4, 2 * f + n % 2, 1))
                return
            x = x_tile(key, 4, 1)
            part = [gate0[tile_rows(j), :] if (f, m) == (0, 0) else gu_acc[m][pl.ds(zero(key, 32), L), :]
                    for m in range(4)]
            gate = _mm(x, weight(wg_v, 4, 1, 2 * f, 2)) + jnp.concatenate(part[:2], axis=1)
            up = _mm(x, weight(wu_v, 4, 1, 2 * f, 2)) + jnp.concatenate(part[2:], axis=1)
            live["h", f] = jnp.maximum(gate, 0.0) * up

        def down(k, n):
            if n == 0:
                live["hidden"] = jnp.concatenate([live.pop(("h", 2 * k + m)) for m in range(2)],
                                                 axis=1).astype(BF16)
            out = _mm(live["hidden"], weight(wd_v, 4 * k, 4, n, 1))
            if k:
                out = out + out_acc[(k + 1) % 2][n][pl.ds(zero(("down", k, n), 32), L), :]
            if k == 2:
                if n == 0:
                    live["rest"] = 1.0 - jnp.broadcast_to(gT[j][0:1], (L, L)).T
                out = out * live["rest"]
            out_acc[k % 2][n][...] = out

        def project(n):
            if n == 0:
                live["o"] = oT[pl.ds(0, 4 * L), :].T.astype(BF16)
            out_acc[1][n][...] = (_mm(live["o"], weight(wo_v, 0, 4, n, 1))
                                  + out_acc[0][n][pl.ds(zero(("wo", n), 32), L), :])

        def finish():
            o = oT[pl.ds(4 * L, L), :].T
            last = jnp.concatenate([
                _mm(o.astype(BF16), weight(wo_v, 4, 1, 0, 4)),
                jnp.concatenate([_mm(o[r:r + 32].astype(BF16), weight(wo_v, 4, 1, 4, 1))
                                 for r in range(0, L, 32)], axis=0)], axis=1)
            out = jnp.concatenate([out_acc[1][n][pl.ds(zero("out", 32), L), :] for n in range(ND)], axis=1)
            out_v[tile_rows(j), :] = (out + last).astype(BF16)

        ffn = []
        for k in range(3):
            ffn += [(gate_up, 2 * k + f, n) for f in range(2) for n in range(5)]
            ffn += [(down, k, n) for n in range(ND)]
        ffn = ffn[1:]
        slots = [(L, 0)] * len(ffn) + [(L, (NI - 1) * NT)] * ND + [(L + 32, NI * NT)]
        ffn += [(project, n) for n in range(ND)] + [(finish,)]
        prog = _plan(slots)
        qk_ends = [task[2] for task in prog if task[0] == "qk"]
        p_next = []
        for kind, *args in prog:
            if kind == "qk":
                mxu_scores(*args)
            elif kind == "ffn":
                run, *where = ffn[args[0]]
                run(*where)
            else:
                weigh_values(*args)
                if args == [NI - 1, NT - 1]:
                    q = q_tile(jnp.minimum(j + 1, NT - 1))
                    for h in range(HT):
                        k = k_ahead.at[pl.ds(zero(("ahead", h), 2), DH)]
                        p, live["link"] = first_keys(q, k, h, always, live["link"], 2)
                        p_next.append(p)
        pltpu.make_async_copy(out_v.at[tile_rows(j)], out_hbm.at[tile_rows(j)], sems.at[10]).start()
        return p_next

    whole_output = pltpu.make_async_copy(out_v, out_hbm, sems.at[10])

    @pl.when(bounded)
    def _():
        lax.fori_loop(0, NT, bounded_tile, [p_first[h] for h in range(HT)])

    @pl.when(jnp.logical_not(bounded))
    def _():
        lax.fori_loop(0, NT, shifted_tile, 0)
        whole_output.start()

    whole_output.wait()


@jax.jit
def pallas_gated_mix__grouped_kv_mqa__glu_gated_reglu__prompt_kernel(
    A_x: jax.Array,
    A_wq: jax.Array,
    A_wk: jax.Array,
    A_wv: jax.Array,
    A_wo: jax.Array,
    B_x: jax.Array,
    B_W_gate: jax.Array,
    B_W_up: jax.Array,
    B_W_down: jax.Array,
    gate_w: jax.Array,
):
    del B_x
    vmem = pltpu.VMEM
    out = pl.pallas_call(
        _kernel,
        out_shape=jax.ShapeDtypeStruct((S, D), BF16),
        in_specs=[pl.BlockSpec(memory_space=pl.ANY)] * 9,
        out_specs=pl.BlockSpec(memory_space=pl.ANY),
        scratch_shapes=[
            vmem((8, DH, D), BF16),
            vmem((8, ND, L), BF16),
            vmem((S // 2, D), U32),
            vmem((D // 2, D), U32),
            vmem((D // 2, D), U32),
            vmem((D // 2, F), U32),
            vmem((D // 2, F), U32),
            vmem((F // 2, D), U32),
            vmem((2 * L, L), U32),
            vmem((ND, 704, L), BF16),
            vmem((NT, D // 2, L), U32),
            vmem((NT * QG, 8, 2 * L), F32),
            vmem((S, L), F32),
            vmem((S // 2, L), U32),
            vmem((-(-NB * 7 * HD // 4) * 4, 24, L), F32),
            vmem((DH, 16, L), F32),
            vmem((NT, VR, L), F32),
            vmem((NT, 8, L), F32),
            vmem((HT, 16, L), F32),
            vmem((NT, H - HT, 16, L), F32),
            vmem((S, L), F32),
            vmem((D + 32, L), F32),
            vmem((S, D), BF16),
            vmem((D + 32, L), F32),
            vmem((S, HG * L), F32),
            pltpu.SemaphoreType.DMA((11,)),
        ] + [vmem((32, L), F32)] * 8 + [vmem((L, L), F32)] * 14,
        compiler_params=pltpu.CompilerParams(vmem_limit_bytes=100 * 2 ** 20),
        name="gated_mix",
    )(A_wk.T, A_wv.T, gate_w.reshape(ND, L), A_x.reshape(S, D), A_wq, A_wo, B_W_gate, B_W_up, B_W_down)
    return out.reshape(1, S, D)
```

```python
import functools
import math

import jax
import jax.numpy as jnp
from jax import lax
import jax.experimental.pallas as pl
import jax.experimental.pallas.tpu as pltpu

S, D, H, DH, F = 2048, 640, 32, 20, 1536
L = 128
NT = S // L
ND = D // L
HG = 4
NI = H // HG
HD = DH // 2
VR = 24
BF16, F32, U32 = jnp.bfloat16, jnp.float32, jnp.uint32

MAX_SCORE = 72.0
MAX_VALUE = 2.0 ** 30

NB = 9
HT = 24
XCH = (2, 4, 10)

VPU_UNITS = [(b, half, a) for b in range(NB) for half in range(2) for a in range(3)]
CUT = [0] + [max(0, (t * (len(VPU_UNITS) + 2) + NT // 2) // NT - 2) for t in range(1, NT + 1)]
VPU_ROWS = [VPU_UNITS[CUT[t]:CUT[t + 1]] for t in range(NT)]
MXU_ROWS = [L - 8 * len(VPU_ROWS[t]) - (16 if t == 0 else 0) for t in range(NT)]
START = [sum(MXU_ROWS[:t]) for t in range(NT + 1)]
PER_ITEM = START[NT]
X_AT = [sum(XCH[:i]) for i in range(len(XCH) + 1)]
QG = D // 8 + 2


def _q_row(head, feature):
    return (feature // HD * 2 + head % 2) * (D // 4) + head // 2 * HD + feature % HD


def _plan(slots, wait=168, min_rows=16, min_gap=96, reserve=6, lag=51.2):
    total = NI * PER_ITEM
    ends = [i * PER_ITEM + START[c + 1] for i in range(NI) for c in range(NT)]
    att_total = total + NI * NT * VR
    ffn_total = sum(cycles for cycles, _ in slots[:len(slots) - reserve])
    prog, ripe, pv_at = [], [], []
    t = att = ffn = row = slot = tile = 0
    while row < total or ripe:
        due = max(ripe[0], pv_at[-1] + min_gap if pv_at else 0) if ripe else None
        if ripe and due <= t:
            ripe.pop(0)
            prog.append(("pv", len(pv_at) // NT, len(pv_at) % NT))
            pv_at.append(t)
            t, att = t + VR, att + VR
            continue
        need = slots[slot][1] if slot < len(slots) else None
        free = need == 0 or (need and len(pv_at) >= need and pv_at[need - 1] + 400 <= t)
        behind = (free and bool(prog) and slot < len(slots) - reserve
                  and (ffn + lag) / ffn_total <= att / att_total)
        if behind and prog[-1][0] == "pv" and row < total:
            n = min_rows
        elif behind or row == total:
            if free:
                prog.append(("ffn", slot))
                t, ffn, slot = t + slots[slot][0], ffn + slots[slot][0], slot + 1
            else:
                t = due
            continue
        elif ripe:
            n = max(min_rows, -(-(due - t) // 16) * 16)
        else:
            n = -(-(ends[tile] - row + wait) // 16) * 16
        n = min(n, total - row)
        prog.append(("qk", row, row + n))
        while tile < len(ends) and ends[tile] <= row + n:
            ripe.append(t + ends[tile] - row + wait)
            tile += 1
        t, att, row = t + n, att + n, row + n
    return prog + [("ffn", n) for n in range(slot, len(slots))]


def _mm(a, b):
    return jnp.dot(a, b, preferred_element_type=F32)


def _unpack(v):
    return pltpu.bitcast(v, BF16)


def _pack(v):
    return pltpu.bitcast(v.astype(BF16), U32)


def _top(acc):
    return functools.reduce(jnp.maximum, [acc[r:r + 8] for r in range(0, acc.shape[0], 8)])


def _kernel(wk_hbm, wv_hbm, gw_hbm, x_hbm, wq_hbm, wo_hbm, wg_hbm, wu_hbm, wd_hbm, out_hbm,
            wkv_v, gw_v, x_v, wq_v, wo_v, wg_v, wu_v, wd_v, wg0_v, wT, xT, q_v, k_all, k_mxu,
            k_vpu, k_ahead, vT, gT, p_first, p_ahead, gate0, oT, out_v, s_v, q_rows, sems, *bufs):
    o_acc, gu_acc, out_acc = (bufs[:4], bufs[4:8]), bufs[8:12], (bufs[12:17], bufs[17:22])

    def fetch(sem, *pairs):
        copies = [pltpu.make_async_copy(src, dst, sems.at[sem]) for src, dst in pairs]
        for c in copies:
            c.start()
        return lambda: [c.wait() for c in copies]

    def x_chunk(i):
        rows = pl.ds(X_AT[i] * L, XCH[i] * L)
        return x_hbm.at[rows], x_v.bitcast(BF16).at[rows]

    small_ready = fetch(0, (wk_hbm, wkv_v.at[0]), (wv_hbm, wkv_v.at[1]), (gw_hbm, gw_v.at[0]))
    x_ready = [fetch(1, x_chunk(0))]
    wq_ready = [fetch(2 + n, (wq_hbm.at[pl.ds(n * L, L)], wq_v.bitcast(BF16).at[pl.ds(n * L, L)]))
                for n in range(ND)]
    x_ready += [fetch(7, x_chunk(1)),
                fetch(8, x_chunk(2), (wg_hbm.at[pl.ds(0, 4 * L), pl.ds(0, L)], wg0_v.bitcast(BF16)))]
    weights_ready = fetch(9, *((src, dst.bitcast(BF16)) for src, dst in (
        (wg_hbm, wg_v), (wu_hbm, wu_v), (wd_hbm, wd_v), (wo_hbm, wo_v))))

    small_ready()
    gw = gw_v[0].astype(F32)
    head = jnp.concatenate([
        wkv_v[0].astype(F32), jnp.zeros((4, D), F32), wkv_v[1].astype(F32),
        jnp.concatenate([gw[n:n + 1] for n in range(ND)], axis=1), jnp.zeros((3, D), F32)], axis=0)
    for n in range(ND):
        wT[n, pl.ds(0, 48), :] = head[:, n * L:(n + 1) * L].astype(BF16)
    nil = pl.multiple_of(jnp.max(jnp.where(gw > jnp.inf, 1.0, 0.0)).astype(jnp.int32) << 5, 32)

    def transpose_x(t):
        xT[t] = _pack(_unpack(x_v[pl.ds(t * L // 2, L // 2), :]).T)

    x_ready[0]()
    for t in range(XCH[0]):
        transpose_x(t)
    order = sorted(range(2 * H), key=lambda a: _q_row(a // 2, a % 2 * HD))
    for n in range(ND):
        wq_ready[n]()
        w = _pack(_unpack(wq_v[pl.ds(n * L // 2, L // 2), :]).T)
        wT[n, pl.ds(48, D), :] = _unpack(jnp.concatenate([w[5 * a:5 * a + 5] for a in order], axis=0))

    def q_tile(j, offset=0):
        return q_v.at[pl.ds(j * QG + offset, QG)]

    def q_feature(q, row, side=0):
        return q[row // 8, pl.ds(row % 8, 1), pl.ds(side * L, L)]

    def chained(always, q_row, link):
        return q_row if link is None else jnp.where(always, q_row, link)

    def times(k, q):
        return k * (q if q.shape[0] == 1 else jnp.concatenate([q] * (k.shape[0] // 8), axis=0))

    def first_keys(q, k, h, always, link, link_at):
        acc = None
        for d in range(DH):
            qd = q_feature(q, _q_row(h, d))
            term = times(k[d], chained(always, qd, link) if d == link_at else qd)
            acc = term if acc is None else acc + term
        return jnp.exp2(acc), _top(acc)

    link = None

    def first_keys_of(t, heads):
        always = q_tile(0)[D // 8, :, pl.ds(0, L)] == 0.0
        out = link
        for h in heads:
            p, out = first_keys(q_tile(t), k_ahead, h, always, out, 0)
            if h < HT:
                p_first[h] = p
            else:
                p_ahead[t, h - HT] = p
        return out

    q_norm = k_norm = v_peak = jnp.zeros((8, L), F32)
    wT32 = wT.bitcast(U32)
    phase = [0, X_AT[1], X_AT[2] - 1, NT]
    for i in range(3):
        if i:
            x_ready[i]()
            if phase[i] == X_AT[i]:
                transpose_x(X_AT[i])
        for t in range(phase[i], phase[i + 1]):
            xt = _unpack(xT[t, pl.ds(nil, D // 2), :])
            if i and t + 1 < X_AT[i + 1]:
                transpose_x(t + 1)
            proj = jnp.concatenate([
                _mm(jnp.concatenate([_unpack(wT32[n, pl.ds(a // 2, (b - a) // 2), :]) for n in range(ND)],
                                    axis=1), xt)
                for a, b in ((0, 176), (176, 352), (352, 528), (528, 48 + D))], axis=0)

            q = proj[48:] * (DH ** -0.5 * math.log2(math.e))
            b11, b12, b21, b22 = (q[m * D // 4:(m + 1) * D // 4] for m in range(4))
            t1 = b12 - b11
            t2 = b22 - t1
            mixed = jnp.concatenate([b21 - t2, t1, t2, b22 - b12], axis=0)
            both = jnp.concatenate([q, mixed], axis=1)
            both = jnp.concatenate([both, jnp.zeros((16, 2 * L), F32)], axis=0)
            q_v[pl.ds(t * QG, QG)] = both.reshape(QG, 8, 2 * L)
            q_rows[t, pl.ds(0, D + 8), :] = both[:D + 8, :L]
            sq = q[:D // 2] * q[:D // 2] + q[D // 2:] * q[D // 2:]
            for h in range(H):
                r = _q_row(h, 0) // 8 * 8
                q_norm = jnp.maximum(q_norm, sq[r:r + 8] + sq[r + 8:r + 16])

            k = proj[:24]
            k_norm = jnp.maximum(k_norm, jnp.sum(k * k, axis=0, keepdims=True))
            k = jnp.concatenate([k[:HD], jnp.zeros((16 - HD, L), F32), k[HD:DH],
                                 jnp.zeros((L - 16 - HD, L), F32)], axis=0).T
            k_all[pl.ds(t * L, L), :] = k
            if t == 0:
                for d in range(DH):
                    e = d // HD * 16 + d % HD
                    k_ahead[d] = jnp.broadcast_to(k[:16, e:e + 1], (16, L))
                k = k[16:]
            if START[t + 1] % 16 == 0:
                u = max(u for u in range(t + 1) if START[u] % 16 == 0)
                rows = [k_all[pl.ds((w + 1) * L - MXU_ROWS[w], MXU_ROWS[w]), :] for w in range(u, t)]
                k_mxu[pl.ds(START[u] // 2, (START[t + 1] - START[u]) // 2), :] = _pack(
                    jnp.concatenate(rows + [k[8 * len(VPU_ROWS[t]):]], axis=0))
            for n, (b, half, a) in enumerate(VPU_ROWS[t]):
                for d in range(HD):
                    lo, hi = (jnp.broadcast_to(k[8 * n:8 * n + 8, e:e + 1], (8, L)) for e in (d, d + 16))
                    at = [((b * 7 + m) * HD + d, pl.ds(8 * a, 8)) for m in range(7)]
                    if half == 0:
                        k_vpu[at[0]], k_vpu[at[1]] = lo, hi
                    else:
                        a11, a12 = k_vpu[at[0]], k_vpu[at[1]]
                        s1 = lo + hi
                        s2 = s1 - a11
                        for m, term in enumerate((a12 - s2, hi, s1, s2, a11 - lo), 2):
                            k_vpu[at[m]] = term

            v = proj[24:48]
            row = lax.broadcasted_iota(jnp.int32, (VR, L), 0)
            gT[t] = jnp.broadcast_to(1.0 / (1.0 + jnp.exp(-v[DH:DH + 1])), (8, L))
            v = jnp.where(row < DH, v, 0.0)
            v_peak = jnp.maximum(v_peak, _top(jnp.abs(v)))
            vT[t] = jnp.where(row < DH, v, 1.0).astype(BF16).astype(F32)
            if t == NT - 1:
                gate0[...] = _mm(_unpack(x_v[:, pl.ds(0, 4 * L)]), _unpack(wg0_v[...]))
            if t:
                link = first_keys_of(t - 1, range(HT, H))
    link = first_keys_of(NT - 1, range(HT, H))
    first_keys_of(0, range(HT))
    v_top = jnp.max(v_peak)
    bounded = ((8.0 * jnp.max(q_norm) * jnp.max(k_norm) <= MAX_SCORE ** 2)
               & (v_top <= MAX_VALUE) & (v_top >= 1.0 / MAX_VALUE))
    weights_ready()

    def head_q(j, i, u):
        return jnp.concatenate([q_rows[j, pl.ds(i * (HG // 2 * HD) + _q_row(u, d), 16), :] for d in (0, HD)],
                               axis=0)

    def store_heads(j, i, heads):
        row = lax.broadcasted_iota(jnp.int32, (8, L), 0)
        total = heads[0][16:]
        for u in range(1, HG):
            total = jnp.where(row == 4 + u, heads[u][16:], total)
        scale = gT[j] / total
        for u in range(HG):
            oT[pl.ds((i * HG + u) * DH, VR), :] = heads[u] * scale[4 + u:5 + u]

    def tile_rows(j, n=L):
        return pl.ds(pl.multiple_of(j * n, n), n)

    def shifted_tile(j, carry):
        def item(i, carry):
            q = jnp.concatenate([head_q(j, i, u) for u in range(HG)], axis=1)
            s = _mm(k_all[...][:, :32].astype(BF16), q.astype(BF16))
            s_v[...] = s
            row_max = jnp.max(s, axis=0, keepdims=True)
            o = _mm(jnp.concatenate([vT[c] for c in range(NT)], axis=1), jnp.exp2(s_v[...] - row_max))
            store_heads(j, i, [o[:, u * L:(u + 1) * L] for u in range(HG)])
            return carry

        lax.fori_loop(0, NI, item, 0)
        x = _unpack(x_v[tile_rows(j, L // 2), :])
        hidden = jnp.maximum(_mm(x, _unpack(wg_v[...])), 0.0) * _mm(x, _unpack(wu_v[...]))
        rest = 1.0 - jnp.broadcast_to(gT[j][0:1], (L, L)).T
        out = (_mm(oT[pl.ds(0, D), :].T.astype(BF16), _unpack(wo_v[...]))
               + jnp.concatenate([rest] * ND, axis=1) * _mm(hidden.astype(BF16), _unpack(wd_v[...])))
        out_v[tile_rows(j), :] = out.astype(BF16)
        return carry

    def bounded_tile(j, p_carry):
        live, zeros = {}, {}
        always = q_tile(j)[D // 8, :, pl.ds(0, L)] == 0.0

        def zero(key, unit):
            if key not in zeros:
                zeros[key] = (j + len(zeros)) >> 13
            return pl.multiple_of(zeros[key] * unit, unit)

        def mxu_scores(row0, row1):
            for i in range(row0 // PER_ITEM, (row1 - 1) // PER_ITEM + 1):
                a, b = max(row0 - i * PER_ITEM, 0), min(row1 - i * PER_ITEM, PER_ITEM)
                for u in range(HG):
                    extra = 16 * (u // 2) if row0 == 0 else 0
                    k = _unpack(k_mxu[pl.ds(zero(i, 32) + a // 2, (b + extra - a) // 2), :])[:, :32]
                    if a == 0:
                        live["q", u] = head_q(j, i, u).astype(BF16)
                    p = jnp.exp2(_mm(k, live["q", u]))
                    for c in range(NT):
                        lo, hi = max(a, START[c]), min(b, START[c + 1])
                        if lo < hi:
                            live.setdefault(("p", i, u, c), []).append(p[lo - a:hi - a])

        def vpu_scores(i, pair, b):
            k = k_vpu.at[pl.ds(zero(("k", i, pair), 4) + b * 7 * HD, 7 * HD)]
            q = q_tile(j, zero(("q", i, b), 2))

            def product(m, acc, link):
                quarter, side = ((0, 2, 3)[m], 0) if m < 3 else (m - 3, 1)
                for d in range(HD):
                    qd = q_feature(q, quarter * (D // 4) + (2 * i + pair) * HD + d, side)
                    term = times(k[m * HD + d], chained(always, qd, link) if d == 3 else qd)
                    acc = term if acc is None else acc + term
                return acc

            p1 = product(0, None, live.get("link"))
            c11 = product(1, p1, None)
            u2 = product(5, p1, _top(c11))
            u3 = product(6, u2, None)
            c21 = product(3, u3, None)
            p5 = product(4, None, _top(c21))
            c12 = product(2, u2 + p5, None)
            live["link"] = _top(c12)
            for half, u, s in ((0, 0, c11), (0, 1, c12), (1, 0, c21), (1, 1, u3 + p5)):
                for a in range(3):
                    live["p", i, 2 * pair + u, b, half, a] = jnp.exp2(s[8 * a:8 * a + 8])

        def weigh_values(i, c):
            v = vT[zero(i, 4) + c]
            for b, half, a in VPU_ROWS[c]:
                if (half, a) == (0, 0):
                    for pair in range(2):
                        vpu_scores(i, pair, b)
            done = []
            for u in range(HG):
                h = i * HG + u
                p = [live.pop(("p", i, u) + unit) for unit in VPU_ROWS[c]] + live.pop(("p", i, u, c))
                if c == 0:
                    p = [p_carry[h] if h < HT else p_ahead[j, h - HT]] + p
                o = _mm(v, jnp.concatenate(p, axis=0))
                if c:
                    o = o + o_acc[(c + 1) % 2][u][pl.ds(zero(i, 32), VR), :]
                if c < NT - 1:
                    o_acc[c % 2][u][pl.ds(0, VR), :] = o
                else:
                    done.append(o)
            if done:
                store_heads(j, i, done)

        def weight(ref, k0, nk, n0, nn):
            return _unpack(ref[pl.ds(k0 * L // 2, nk * L // 2), pl.ds(n0 * L, nn * L)])

        def x_tile(key, k0, nk):
            rows = pl.ds(pl.multiple_of(zero(key, 32) + j * (L // 2), 32), L // 2)
            return _unpack(x_v[rows, pl.ds(k0 * L, nk * L)])

        def gate_up(f, n):
            key = ("gu", f, n)
            if n < 4:
                gu_acc[n][...] = _mm(x_tile(key, 0, 4), weight((wg_v, wu_v)[n // 2], 0, 4, 2 * f + n % 2, 1))
                return
            x = x_tile(key, 4, 1)
            part = [gate0[tile_rows(j), :] if (f, m) == (0, 0) else gu_acc[m][pl.ds(zero(key, 32), L), :]
                    for m in range(4)]
            gate = _mm(x, weight(wg_v, 4, 1, 2 * f, 2)) + jnp.concatenate(part[:2], axis=1)
            up = _mm(x, weight(wu_v, 4, 1, 2 * f, 2)) + jnp.concatenate(part[2:], axis=1)
            live["h", f] = jnp.maximum(gate, 0.0) * up

        def down(k, n):
            if n == 0:
                live["hidden"] = jnp.concatenate([live.pop(("h", 2 * k + m)) for m in range(2)],
                                                 axis=1).astype(BF16)
            out = _mm(live["hidden"], weight(wd_v, 4 * k, 4, n, 1))
            if k:
                out = out + out_acc[(k + 1) % 2][n][pl.ds(zero(("down", k, n), 32), L), :]
            if k == 2:
                if n == 0:
                    live["rest"] = 1.0 - jnp.broadcast_to(gT[j][0:1], (L, L)).T
                out = out * live["rest"]
            out_acc[k % 2][n][...] = out

        def project(n):
            if n == 0:
                live["o"] = oT[pl.ds(0, 4 * L), :].T.astype(BF16)
            out_acc[1][n][...] = (_mm(live["o"], weight(wo_v, 0, 4, n, 1))
                                  + out_acc[0][n][pl.ds(zero(("wo", n), 32), L), :])

        def finish():
            o = oT[pl.ds(4 * L, L), :].T
            last = jnp.concatenate([
                _mm(o.astype(BF16), weight(wo_v, 4, 1, 0, 4)),
                jnp.concatenate([_mm(o[a:b].astype(BF16), weight(wo_v, 4, 1, 4, 1))
                                 for a, b in ((0, 48), (48, 80), (80, 112), (112, L))], axis=0)], axis=1)
            out = jnp.concatenate([out_acc[1][n][pl.ds(zero("out", 32), L), :] for n in range(ND)], axis=1)
            out_v[tile_rows(j), :] = (out + last).astype(BF16)

        ffn = []
        for k in range(3):
            ffn += [(gate_up, 2 * k + f, n) for f in range(2) for n in range(5)]
            ffn += [(down, k, n) for n in range(ND)]
        ffn = ffn[1:]
        slots = [(L, 0)] * len(ffn) + [(L, (NI - 1) * NT)] * ND + [(L + 32, NI * NT)]
        ffn += [(project, n) for n in range(ND)] + [(finish,)]
        p_next = []
        for kind, *args in _plan(slots):
            if kind == "qk":
                mxu_scores(*args)
            elif kind == "ffn":
                run, *where = ffn[args[0]]
                run(*where)
            else:
                weigh_values(*args)
                if args == [NI - 1, NT - 1]:
                    q = q_tile(jnp.minimum(j + 1, NT - 1))
                    for h in range(HT):
                        k = k_ahead.at[pl.ds(zero(("ahead", h), 2), DH)]
                        p, live["link"] = first_keys(q, k, h, always, live["link"], 2)
                        p_next.append(p)
        pltpu.make_async_copy(out_v.at[tile_rows(j)], out_hbm.at[tile_rows(j)], sems.at[10]).start()
        return p_next

    whole_output = pltpu.make_async_copy(out_v, out_hbm, sems.at[10])

    @pl.when(bounded)
    def _():
        lax.fori_loop(0, NT, bounded_tile, [p_first[h] for h in range(HT)])

    @pl.when(jnp.logical_not(bounded))
    def _():
        lax.fori_loop(0, NT, shifted_tile, 0)
        whole_output.start()

    whole_output.wait()


@jax.jit
def pallas_gated_mix__grouped_kv_mqa__glu_gated_reglu__prompt_kernel(
    A_x: jax.Array,
    A_wq: jax.Array,
    A_wk: jax.Array,
    A_wv: jax.Array,
    A_wo: jax.Array,
    B_x: jax.Array,
    B_W_gate: jax.Array,
    B_W_up: jax.Array,
    B_W_down: jax.Array,
    gate_w: jax.Array,
):
    del B_x
    vmem = pltpu.VMEM
    out = pl.pallas_call(
        _kernel,
        out_shape=jax.ShapeDtypeStruct((S, D), BF16),
        in_specs=[pl.BlockSpec(memory_space=pl.ANY)] * 9,
        out_specs=pl.BlockSpec(memory_space=pl.ANY),
        scratch_shapes=[
            vmem((8, DH, D), BF16),
            vmem((8, ND, L), BF16),
            vmem((S // 2, D), U32),
            vmem((D // 2, D), U32),
            vmem((D // 2, D), U32),
            vmem((D // 2, F), U32),
            vmem((D // 2, F), U32),
            vmem((F // 2, D), U32),
            vmem((2 * L, L), U32),
            vmem((ND, 704, L), BF16),
            vmem((NT, D // 2, L), U32),
            vmem((NT * QG, 8, 2 * L), F32),
            vmem((S, L), F32),
            vmem((S // 2, L), U32),
            vmem((-(-NB * 7 * HD // 4) * 4, 24, L), F32),
            vmem((DH, 16, L), F32),
            vmem((NT, VR, L), F32),
            vmem((NT, 8, L), F32),
            vmem((HT, 16, L), F32),
            vmem((NT, H - HT, 16, L), F32),
            vmem((S, L), F32),
            vmem((D + 32, L), F32),
            vmem((S, D), BF16),
            vmem((S, HG * L), F32),
            vmem((NT, D + 32, L), F32),
            pltpu.SemaphoreType.DMA((11,)),
        ] + [vmem((32, L), F32)] * 8 + [vmem((L, L), F32)] * 14,
        compiler_params=pltpu.CompilerParams(vmem_limit_bytes=100 * 2 ** 20),
        name="gated_mix",
    )(A_wk.T, A_wv.T, gate_w.reshape(ND, L), A_x.reshape(S, D), A_wq, A_wo, B_W_gate, B_W_up, B_W_down)
    return out.reshape(1, S, D)
```
